```python
import jax
import jax.numpy as jnp

def _softmax(x, axis=-1):
    return jax.nn.softmax(x, axis=axis)

def _gelu(x):
    return jax.nn.gelu(x, approximate=True)

def _silu(x):
    return jax.nn.silu(x)

def _sigmoid(x):
    return jax.nn.sigmoid(x)

def _layernorm(x, axis=-1, eps=1e-05):
    m = jnp.mean(x, axis=axis, keepdims=True)
    v = jnp.var(x, axis=axis, keepdims=True)
    return (x - m) / jnp.sqrt(v + eps)

def _scatter_add(tgt, idx, src, axis=0):
    return tgt.at[idx].add(src)

def _segment_sum(src, seg, n):
    return jax.ops.segment_sum(src, seg, n)

class _Rng:

    def __init__(self, key):
        self._k = key

    def _next(self):
        self._k, sub = jax.random.split(self._k)
        return sub

    def normal(self, shape):
        return jax.random.normal(self._next(), shape, dtype=jnp.bfloat16)

    def randint(self, lo, hi, shape):
        return jax.random.randint(self._next(), shape, lo, hi, dtype=jnp.int32)

    def uniform(self, shape, lo=0.0, hi=1.0):
        return jax.random.uniform(self._next(), shape, jnp.bfloat16, lo, hi)

    def permutation(self, n):
        return jax.random.permutation(self._next(), n)
kernel_name = 'standalone__window_attn_davit__vision'

def setup_inputs():
    _rng = _Rng(jax.random.key(int.from_bytes(__import__("os").urandom(4), "little")))
    _w = lambda a: (lambda t: t.astype(jnp.bfloat16) if jnp.issubdtype(t.dtype, jnp.floating) else t)(jnp.asarray(a))
    HW = 512
    C0 = 192
    ws = 7
    nh = 4
    H = W = max(HW // ws * ws, ws)
    C = max(C0 // nh * nh, nh)
    k = 3
    return {'x': _w((lambda *s: _rng.normal(s) * 0.05)(1, H, W, C)), 'dw_pe': _w((lambda *s: _rng.normal(s) * 0.05)(k, k, C) * 0.1), 'w_qkv': _w((lambda *s: _rng.normal(s) * 0.05)(C, 3 * C) * C ** (-0.5)), 'w_o': _w((lambda *s: _rng.normal(s) * 0.05)(C, C) * C ** (-0.5))}

def reference(x, dw_pe, w_qkv, w_o):
    B, H, W, C = x.shape
    ws = 7
    nh = 4
    dh = C // nh
    kk = dw_pe.shape[0]
    pad = kk // 2
    xp = jnp.pad(x, ((0, 0), (pad, pad), (pad, pad), (0, 0)))
    pe = jnp.zeros_like(x)
    for i in range(kk):
        for j in range(kk):
            pe = pe + xp[:, i:i + H, j:j + W, :] * dw_pe[i, j][None, None, None, :]
    x0 = x + pe
    h = _layernorm(x0, axis=-1)
    hw = h.reshape(B, H // ws, ws, W // ws, ws, C)
    hw = (lambda x, *d: x.transpose(*d))(hw, 0, 1, 3, 2, 4, 5)
    hw = hw.reshape(-1, ws * ws, C)
    qkv = (hw @ w_qkv).reshape(-1, ws * ws, 3, nh, dh)
    q = qkv[:, :, 0].copy()
    k = qkv[:, :, 1].copy()
    v = qkv[:, :, 2].copy()
    scale = dh ** (-0.5)
    attn = jnp.einsum('wnhd,wmhd->whnm', q, k) * scale
    attn = _softmax(attn, axis=-1)
    out = jnp.einsum('whnm,wmhd->wnhd', attn, v)
    out = out.reshape(-1, ws * ws, C) @ w_o
    out = out.reshape(B, H // ws, W // ws, ws, ws, C)
    out = (lambda x, *d: x.transpose(*d))(out, 0, 1, 3, 2, 4, 5)
    out = out.reshape(B, H, W, C)
    return x0 + out
```

```python
import functools

import jax
import jax.numpy as jnp
import jax.experimental.pallas as pl
import jax.experimental.pallas.tpu as pltpu
from jax import lax

WS = 7
NH = 4
C = 192
DH = C // NH
CW = C // 2
F32 = jnp.float32
BF16 = jnp.bfloat16
U32 = jnp.uint32
NT_DIMS = (((1,), (1,)), ((), ()))
NN_DIMS = (((1,), (0,)), ((), ()))
NEG = -1e30
LOG2E = 1.4426950408889634
import os
UW = int(os.environ.get('UW', 8))
UC = int(os.environ.get('UC', 2))
EXACT = bool(int(os.environ.get('EXACT', 0)))
APPROX = bool(int(os.environ.get('APPROX', 0)))


def _dot(a, b, dims=NN_DIMS):
    return lax.dot_general(a, b, dims, preferred_element_type=F32)


def _iota(shape, dim):
    return lax.broadcasted_iota(jnp.int32, shape, dim)


def _f32(words):
    return pltpu.bitcast(words, F32)


def _lo(words):
    return _f32(words << 16)


def _hi(words):
    return _f32(words & U32(0xFFFF0000))


def _pack2(a, b):
    return pltpu.pack_elementwise([a, b], packed_dtype=BF16)


def _onehot(rows_map, cols_map):
    return jnp.where(rows_map == cols_map, 1.0, 0.0).astype(BF16)


def _prepare_weights(dw_ref, wqkv_ref, wo_ref, dwt_ref, wq_ref, wot_ref):
    r_i = _iota((CW, C), 0)
    c_i = _iota((CW, C), 1)
    for p in range(2):
        sel = _onehot(2 * r_i + p, c_i)
        for k in range(9):
            rep = jnp.broadcast_to(dw_ref[k:k + 1, :], (128, C))
            t = _dot(sel, rep, NT_DIMS)
            if k == 4:
                t = t + 1.0
            dwt_ref[k, p] = t
    rho = _iota((256, C), 0)
    rr = rho & 127
    chan = jnp.where(rr < CW, 2 * rr + (rho >> 7), -1)
    rsel = _onehot(chan, _iota((256, C), 1))
    w1 = _dot(rsel, wqkv_ref[...]).astype(BF16)
    n = _iota((3 * C, 640), 1)
    l = n & 127
    t = n >> 7
    col0 = jnp.where(l < 96, l, 384 + 64 + l - 96)
    col1 = jnp.where(l >= 32, 96 + l - 32, 384 + l)
    col2 = jnp.where(l < 96, 192 + l, -1)
    col3 = jnp.where(l >= 32, 288 + l - 32, -1)
    col4 = jnp.where(l < 32, 480 + l, jnp.where(l < 64, 384 + l, 448 + l))
    col = jnp.where(t == 0, col0, jnp.where(t == 1, col1, jnp.where(t == 2, col2,
                    jnp.where(t == 3, col3, col4))))
    csel = _onehot(_iota((3 * C, 640), 0), col)
    wq = _dot(w1, csel)
    wq_ref[...] = pltpu.bitcast(wq.astype(BF16), U32)
    lam = _iota((256, C), 0)
    ll = lam & 127
    fa = jnp.where(ll < 64, ll, jnp.where(ll < 96, -1, ll - 32))
    fb = jnp.where(ll < 32, 96 + ll, jnp.where(ll < 64, -1, 64 + ll))
    feat = jnp.where(lam < 128, fa, fb)
    fsel = _onehot(feat, _iota((256, C), 1))
    tmp = _dot(fsel, wo_ref[...]).astype(BF16)
    rp = _iota((C, C), 0)
    ochan = jnp.where(rp < CW, 2 * rp, 2 * (rp - CW) + 1)
    osel = _onehot(ochan, _iota((C, C), 1))
    wot_ref[...] = pltpu.bitcast(_dot(osel, tmp, NT_DIMS).astype(BF16), U32)


def _kernel(xm_ref, xt_ref, xb_ref, dw_ref, wqkv_ref, wo_ref, o_ref,
            dwt_ref, wq_ref, wot_ref, x0_ref, hs_ref, qkv_ref, os_ref, *, n_strips, width):
    a = pl.program_id(0)
    WP = 512

    @pl.when(a == 0)
    def _():
        _prepare_weights(dw_ref, wqkv_ref, wo_ref, dwt_ref, wq_ref, wot_ref)

    sub = _iota((8, 128), 0)
    lane = _iota((8, 128), 1)
    lo16, hi16 = U32(0x0000FFFF), U32(0xFFFF0000)
    zero = U32(0)

    def rows(m, n):
        return jnp.concatenate([m] * n, axis=0)

    def halves(hp0, hp1):
        return jnp.where(hp0, lo16, jnp.where(hp1, hi16, zero))

    key_ok = sub < WS
    kmask = [halves(lane < 48, (lane >= 48) & (lane < 96)),
             halves((lane >= 32) & (lane < 80), lane >= 80)]
    va1 = ((lane >= 48) & (lane < 64)) | (lane >= 96)
    vb1 = lane >= 80
    vmask = [jnp.where(key_ok, halves(lane < 48, va1), zero),
             jnp.where(key_ok, halves((lane < 32) | ((lane >= 64) & (lane < 80)), vb1), zero)]
    one_lo, one_hi = U32(0x00003F80), U32(0x3F800000)

    def ones(d0):
        m = jnp.where((lane >= d0) & (lane < d0 + 16), one_lo,
                      jnp.where((lane >= d0 + 16) & (lane < d0 + 32), one_hi, zero))
        return jnp.where(key_ok, m, zero)

    vones = [ones(64), ones(32)]
    den_idx = [jnp.where(va1, 80, 64), jnp.where(vb1, 48, 32)]
    even = (lane & 1) == 0
    s_valid = ((lane & 15) < 14) & (lane < 112)
    quarter = lane >> 5
    last_valid = lane < (width - 384)
    c_exp = (DH ** -0.5) * LOG2E

    def conv_group(g, top_ok, bot_ok):
        c0 = pl.multiple_of(g * 16, 16)
        r0 = pl.multiple_of(g * 8, 8)
        taps = [[jnp.concatenate([dwt_ref[k, p, pl.ds(r0, 8), :]] * 4, axis=1)
                 for p in range(2)] for k in range(9)]
        acc = {}
        for r in range(-1, WS + 1):
            if r == -1:
                raw = xt_ref[0, pl.ds(c0, 16), :]
            elif r == WS:
                raw = xb_ref[0, pl.ds(c0, 16), :]
            else:
                raw = xm_ref[r, pl.ds(c0, 16), :]
            w = pltpu.bitcast(raw, U32)
            w = jnp.concatenate([w[:, :384], jnp.where(last_valid, w[:, 384:], zero)], axis=1)
            if r == -1:
                w = jnp.where(top_ok, w, zero)
            if r == WS:
                w = jnp.where(bot_ok, w, zero)
            sh = [pltpu.roll(w, 1, 1), w, pltpu.roll(w, WP - 1, 1)]
            for p, unp in enumerate((_lo, _hi)):
                u = [unp(s) for s in sh]
                for i in range(3):
                    orow = r + 1 - i
                    if orow < 0 or orow >= WS:
                        continue
                    t = u[0] * taps[3 * i][p] + u[1] * taps[3 * i + 1][p] + u[2] * taps[3 * i + 2][p]
                    key = (orow, p)
                    acc[key] = t if key not in acc else acc[key] + t
                    if i == 2:
                        x0_ref[orow, p, pl.ds(r0, 8), :] = acc.pop(key)

    def ln_tile(it):
        i = it >> 2
        l0 = pl.multiple_of((it & 3) * 128, 128)
        xe = x0_ref[i, 0, :, pl.ds(l0, 128)]
        xo = x0_ref[i, 1, :, pl.ds(l0, 128)]
        mean = jnp.sum(xe + xo, axis=0, keepdims=True) * (1.0 / C)
        de = xe - mean
        do = xo - mean
        var = jnp.sum(de * de + do * do, axis=0, keepdims=True) * (1.0 / C)
        rstd = lax.rsqrt(var + 1e-5)
        words = _pack2(de * rstd, do * rstd)
        words = jnp.concatenate([words, jnp.zeros((128 - CW, 128), U32)], axis=0)
        hs_ref[i, pl.ds(l0, 128), :] = words.T

    def qkv_tile(it):
        i = it >> 2
        l0 = pl.multiple_of((it & 3) * 128, 128)
        words = hs_ref[i, pl.ds(l0, 128), :]
        he, ho = _lo(words), _hi(words)
        t = []
        for j in range(5):
            we = pltpu.bitcast(wq_ref[0:64, 128 * j:128 * (j + 1)], BF16)
            wo = pltpu.bitcast(wq_ref[64:128, 128 * j:128 * (j + 1)], BF16)
            t.append(_dot(he, we) + _dot(ho, wo))
        q16 = rows(quarter, 16)
        va = jnp.where(q16 == 0, t[1], jnp.where(q16 == 3, t[0], t[4]))
        res = [pltpu.bitcast(t[0], U32), pltpu.bitcast(t[1], U32),
               _pack2(t[2], t[2]) & rows(kmask[0], 16), _pack2(t[3], t[3]) & rows(kmask[1], 16),
               _pack2(va, va), _pack2(t[4], t[4])]
        for j in range(6):
            qkv_ref[i, j, pl.ds(l0, 128), :] = res[j]

    zpad = jnp.zeros((16, 128), BF16)

    def gather(j, off):
        return jnp.concatenate([qkv_ref[i, j, pl.ds(off, 8), :] for i in range(WS)], axis=0)

    def scores(off, exact_max):
        ps = []
        for pr in range(2):
            q = _f32(gather(pr, off))
            kbd = jnp.concatenate([pltpu.bitcast(gather(2 + pr, off), BF16), zpad], axis=0)
            s = _dot(q, kbd, NT_DIMS)
            if exact_max:
                s = jnp.where(rows(s_valid, WS), s, NEG)
                ev = rows(even, WS)
                m0 = jnp.max(jnp.where(ev, s, NEG), axis=1, keepdims=True)
                m1 = jnp.max(jnp.where(ev, NEG, s), axis=1, keepdims=True)
                s = s - jnp.where(ev, m0, m1)
            ps.append(jnp.exp2(s * c_exp))
        return ps

    def attend(off, ps):
        for pr in range(2):
            vw = (gather(4 + pr, off) & rows(vmask[pr], WS)) | rows(vones[pr], WS)
            vbd = jnp.concatenate([pltpu.bitcast(vw, BF16), zpad], axis=0)
            o = _dot(ps[pr], vbd)
            den = jnp.take_along_axis(o, rows(den_idx[pr], WS), axis=1, mode="promise_in_bounds")
            o = o * pltpu.reciprocal(den, approx=APPROX, full_range=False)
            for i in range(WS):
                os_ref[i, pr, pl.ds(off, 8), :] = o[8 * i:8 * i + 8, :]

    n_win = width // WS

    def attention(exact_max):
        def body(qi, ps):
            base = pl.multiple_of(qi * (UW * WS), 8)
            for u in range(UW):
                nxt = scores(base + WS * (u + 1), exact_max)
                attend(base + WS * u, ps)
                ps = nxt
            return ps
        n_it = (n_win - 1) // UW
        ps = lax.fori_loop(0, n_it, body, scores(0, exact_max))
        for w in range(n_it * UW, n_win):
            nxt = scores(WS * (w + 1), exact_max) if w + 1 < n_win else None
            attend(WS * w, ps)
            ps = nxt

    def out_tile(it):
        i = it >> 2
        l0 = pl.multiple_of((it & 3) * 128, 128)
        oa = os_ref[i, 0, pl.ds(l0, 128), :].astype(BF16)
        ob = os_ref[i, 1, pl.ds(l0, 128), :].astype(BF16)
        wa = pltpu.bitcast(wot_ref[:, 0:128], BF16)
        wb = pltpu.bitcast(wot_ref[:, 128:256], BF16)
        y = _dot(wa, oa, NT_DIMS) + _dot(wb, ob, NT_DIMS)
        ye = y[0:CW] + x0_ref[i, 0, :, pl.ds(l0, 128)]
        yo = y[CW:C] + x0_ref[i, 1, :, pl.ds(l0, 128)]
        o_ref[i, :, pl.ds(l0, 128)] = pltpu.bitcast(_pack2(ye, yo), BF16)

    top_ok = a > 0
    bot_ok = a < n_strips - 1

    def conv_body(g, c):
        conv_group(g, top_ok, bot_ok)
        return c
    lax.fori_loop(0, CW // 8, conv_body, 0)

    ln_tile(0)

    def b_body(it, c):
        ln_tile(jnp.minimum(it + 1, WS * 4 - 1))
        qkv_tile(it)
        return c
    lax.fori_loop(0, WS * 4, b_body, 0)

    attention(EXACT)

    def c_body(it, c):
        for u in range(UC):
            out_tile(it * UC + u)
        return c
    lax.fori_loop(0, WS * 4 // UC, c_body, 0)


@jax.jit
def pallas_standalone__window_attn_davit__vision_kernel(
    x: jax.Array,
    dw_pe: jax.Array,
    w_qkv: jax.Array,
    w_o: jax.Array,
):
    B, H, W, Cc = x.shape
    assert B == 1 and Cc == C and dw_pe.shape == (3, 3, C)
    assert H % WS == 0 and W % WS == 0 and 384 < W <= 512
    n_strips = H // WS
    xt = jnp.transpose(x, (0, 1, 3, 2)).reshape(H, C, W)
    dw = dw_pe.reshape(9, C)

    full = lambda shape: pl.BlockSpec(shape, lambda a: (0,) * len(shape))
    out = pl.pallas_call(
        functools.partial(_kernel, n_strips=n_strips, width=W),
        grid=(n_strips,),
        in_specs=[
            pl.BlockSpec((WS, C, 512), lambda a: (a, 0, 0)),
            pl.BlockSpec((1, C, 512), lambda a: (jnp.maximum(a * WS - 1, 0), 0, 0)),
            pl.BlockSpec((1, C, 512), lambda a: (jnp.minimum(a * WS + WS, H - 1), 0, 0)),
            full((9, C)),
            full((C, 3 * C)),
            full((C, C)),
        ],
        out_specs=pl.BlockSpec((WS, C, 512), lambda a: (a, 0, 0)),
        out_shape=jax.ShapeDtypeStruct((H, C, W), x.dtype),
        scratch_shapes=[
            pltpu.VMEM((9, 2, CW, 128), F32),
            pltpu.VMEM((128, 640), U32),
            pltpu.VMEM((CW, 256), U32),
            pltpu.VMEM((WS, 2, CW, 512), F32),
            pltpu.VMEM((WS, 512, 128), U32),
            pltpu.VMEM((WS, 6, 512, 128), U32),
            pltpu.VMEM((WS, 2, 512, 128), F32),
        ],
        compiler_params=pltpu.CompilerParams(
            dimension_semantics=("arbitrary",),
            vmem_limit_bytes=100 * 1024 * 1024,
        ),
    )(xt, xt, xt, dw, w_qkv, w_o)
    return jnp.transpose(out.reshape(B, H, C, W), (0, 1, 3, 2))
```

```python
import functools

import jax
import jax.numpy as jnp
import jax.experimental.pallas as pl
import jax.experimental.pallas.tpu as pltpu
from jax import lax

WS = 7
NH = 4
C = 192
DH = C // NH
CW = C // 2
F32 = jnp.float32
BF16 = jnp.bfloat16
U32 = jnp.uint32
NT_DIMS = (((1,), (1,)), ((), ()))
NN_DIMS = (((1,), (0,)), ((), ()))
NEG = -1e30
LOG2E = 1.4426950408889634
UW = 8
SKEW = 1
LEAD = 2
EXP_LIMIT = 40.0
UC = 2
APPROX = False


def _dot(a, b, dims=NN_DIMS):
    return lax.dot_general(a, b, dims, preferred_element_type=F32)


def _iota(shape, dim):
    return lax.broadcasted_iota(jnp.int32, shape, dim)


def _f32(words):
    return pltpu.bitcast(words, F32)


def _lo(words):
    return _f32(words << 16)


def _hi(words):
    return _f32(words & U32(0xFFFF0000))


def _pack2(a, b):
    return pltpu.pack_elementwise([a, b], packed_dtype=BF16)


def _onehot(rows_map, cols_map):
    return jnp.where(rows_map == cols_map, 1.0, 0.0).astype(BF16)


def _prepare_weights(dw_ref, wqkv_ref, wo_ref, dwt_ref, wq_ref, wot_ref):
    r_i = _iota((CW, C), 0)
    c_i = _iota((CW, C), 1)
    for p in range(2):
        sel = _onehot(2 * r_i + p, c_i)
        for k in range(9):
            rep = jnp.broadcast_to(dw_ref[k:k + 1, :], (128, C))
            t = _dot(sel, rep, NT_DIMS)
            if k == 4:
                t = t + 1.0
            dwt_ref[k, p] = t
    rho = _iota((256, C), 0)
    rr = rho & 127
    chan = jnp.where(rr < CW, 2 * rr + (rho >> 7), -1)
    rsel = _onehot(chan, _iota((256, C), 1))
    w1 = _dot(rsel, wqkv_ref[...]).astype(BF16)
    n = _iota((3 * C, 640), 1)
    l = n & 127
    t = n >> 7
    col0 = jnp.where(l < 96, l, 384 + 64 + l - 96)
    col1 = jnp.where(l >= 32, 96 + l - 32, 384 + l)
    col2 = jnp.where(l < 96, 192 + l, -1)
    col3 = jnp.where(l >= 32, 288 + l - 32, -1)
    col4 = jnp.where(l < 32, 480 + l, jnp.where(l < 64, 384 + l, 448 + l))
    col = jnp.where(t == 0, col0, jnp.where(t == 1, col1, jnp.where(t == 2, col2,
                    jnp.where(t == 3, col3, col4))))
    csel = _onehot(_iota((3 * C, 640), 0), col)
    wq = _dot(w1, csel)
    wq_ref[...] = pltpu.bitcast(wq.astype(BF16), U32)
    lam = _iota((256, C), 0)
    ll = lam & 127
    fa = jnp.where(ll < 64, ll, jnp.where(ll < 96, -1, ll - 32))
    fb = jnp.where(ll < 32, 96 + ll, jnp.where(ll < 64, -1, 64 + ll))
    feat = jnp.where(lam < 128, fa, fb)
    fsel = _onehot(feat, _iota((256, C), 1))
    tmp = _dot(fsel, wo_ref[...]).astype(BF16)
    rp = _iota((C, C), 0)
    ochan = jnp.where(rp < CW, 2 * rp, 2 * (rp - CW) + 1)
    osel = _onehot(ochan, _iota((C, C), 1))
    wot_ref[...] = pltpu.bitcast(_dot(osel, tmp, NT_DIMS).astype(BF16), U32)


def _kernel(xm_ref, xt_ref, xb_ref, dw_ref, wqkv_ref, wo_ref, o_ref,
            dwt_ref, wq_ref, wot_ref, x0_ref, res_ref, hs_ref, qkv_ref, os_ref, flag_ref,
            *, n_strips, width):
    s = pl.program_id(0)
    WP = 512
    NTILE = WS * 4

    sub = _iota((8, 128), 0)
    lane = _iota((8, 128), 1)
    lo16, hi16 = U32(0x0000FFFF), U32(0xFFFF0000)
    zero = U32(0)

    def rows(m, n):
        return jnp.concatenate([m] * n, axis=0)

    def halves(hp0, hp1):
        return jnp.where(hp0, lo16, jnp.where(hp1, hi16, zero))

    key_ok = sub < WS
    kmask = [halves(lane < 48, (lane >= 48) & (lane < 96)),
             halves((lane >= 32) & (lane < 80), lane >= 80)]
    va1 = ((lane >= 48) & (lane < 64)) | (lane >= 96)
    vb1 = lane >= 80
    vmask = [jnp.where(key_ok, halves(lane < 48, va1), zero),
             jnp.where(key_ok, halves((lane < 32) | ((lane >= 64) & (lane < 80)), vb1), zero)]
    one_lo, one_hi = U32(0x00003F80), U32(0x3F800000)

    def ones(d0):
        m = jnp.where((lane >= d0) & (lane < d0 + 16), one_lo,
                      jnp.where((lane >= d0 + 16) & (lane < d0 + 32), one_hi, zero))
        return jnp.where(key_ok, m, zero)

    vones = [ones(64), ones(32)]
    den_idx = [jnp.where(va1, 80, 64), jnp.where(vb1, 48, 32)]
    even = (lane & 1) == 0
    s_valid = ((lane & 15) < 14) & (lane < 112)
    quarter = lane >> 5
    last_valid = lane < (width - 384)
    c_exp = (DH ** -0.5) * LOG2E

    def conv_group(g):
        top_ok = s > 0
        bot_ok = s < n_strips - 1
        c0 = g * 16 if isinstance(g, int) else pl.multiple_of(g * 16, 16)
        r0 = g * 8 if isinstance(g, int) else pl.multiple_of(g * 8, 8)
        taps = [[jnp.concatenate([dwt_ref[k, p, pl.ds(r0, 8), :]] * 4, axis=1)
                 for p in range(2)] for k in range(9)]
        acc = {}
        for r in range(-1, WS + 1):
            if r == -1:
                raw = xt_ref[0, pl.ds(c0, 16), :]
            elif r == WS:
                raw = xb_ref[0, pl.ds(c0, 16), :]
            else:
                raw = xm_ref[r, pl.ds(c0, 16), :]
            w = pltpu.bitcast(raw, U32)
            w = jnp.concatenate([w[:, :384], jnp.where(last_valid, w[:, 384:], zero)], axis=1)
            if r == -1:
                w = jnp.where(top_ok, w, zero)
            if r == WS:
                w = jnp.where(bot_ok, w, zero)
            sh = [pltpu.roll(w, 1, 1), w, pltpu.roll(w, WP - 1, 1)]
            for p, unp in enumerate((_lo, _hi)):
                u = [unp(t) for t in sh]
                for i in range(3):
                    orow = r + 1 - i
                    if orow < 0 or orow >= WS:
                        continue
                    t = u[0] * taps[3 * i][p] + u[1] * taps[3 * i + 1][p] + u[2] * taps[3 * i + 2][p]
                    key = (orow, p)
                    acc[key] = t if key not in acc else acc[key] + t
                    if i == 2:
                        x0_ref[orow, p, pl.ds(r0, 8), :] = acc.pop(key)

    def tile_pos(it):
        if isinstance(it, int):
            return it // 4, (it % 4) * 128
        return it >> 2, pl.multiple_of((it & 3) * 128, 128)

    def ln_tile(it):
        i, l0 = tile_pos(it)
        xe = x0_ref[i, 0, :, pl.ds(l0, 128)]
        xo = x0_ref[i, 1, :, pl.ds(l0, 128)]
        res_ref[i, :, pl.ds(l0, 128)] = _pack2(xe, xo)
        mean = jnp.sum(xe + xo, axis=0, keepdims=True) * (1.0 / C)
        de = xe - mean
        do = xo - mean
        var = jnp.sum(de * de + do * do, axis=0, keepdims=True) * (1.0 / C)
        rstd = lax.rsqrt(var + 1e-5)
        words = _pack2(de * rstd, do * rstd)
        words = jnp.concatenate([words, jnp.zeros((128 - CW, 128), U32)], axis=0)
        hs_ref[i, pl.ds(l0, 128), :] = words.T

    def qkv_tile(it):
        i, l0 = tile_pos(it)
        words = hs_ref[i, pl.ds(l0, 128), :]
        he, ho = _lo(words), _hi(words)
        t = []
        for j in range(5):
            we = pltpu.bitcast(wq_ref[0:64, 128 * j:128 * (j + 1)], BF16)
            wo = pltpu.bitcast(wq_ref[64:128, 128 * j:128 * (j + 1)], BF16)
            t.append(_dot(he, we) + _dot(ho, wo))
        q16 = rows(quarter, 16)
        va = jnp.where(q16 == 0, t[1], jnp.where(q16 == 3, t[0], t[4]))
        res = [pltpu.bitcast(t[0], U32), pltpu.bitcast(t[1], U32),
               _pack2(t[2], t[2]) & rows(kmask[0], 16), _pack2(t[3], t[3]) & rows(kmask[1], 16),
               _pack2(va, va), _pack2(t[4], t[4])]
        for j in range(6):
            qkv_ref[i, j, pl.ds(l0, 128), :] = res[j]

    zpad = jnp.zeros((16, 128), BF16)

    def gather(j, off):
        return jnp.concatenate([qkv_ref[i, j, pl.ds(off, 8), :] for i in range(WS)], axis=0)

    def scores(off, exact_max):
        ps = []
        for pr in range(2):
            q = _f32(gather(pr, off))
            kbd = jnp.concatenate([pltpu.bitcast(gather(2 + pr, off), BF16), zpad], axis=0)
            sc = _dot(q, kbd, NT_DIMS)
            if exact_max:
                sc = jnp.where(rows(s_valid, WS), sc, NEG)
                ev = rows(even, WS)
                m0 = jnp.max(jnp.where(ev, sc, NEG), axis=1, keepdims=True)
                m1 = jnp.max(jnp.where(ev, NEG, sc), axis=1, keepdims=True)
                sc = sc - jnp.where(ev, m0, m1)
            ps.append(jnp.exp2(sc * c_exp))
        return ps

    def attend(off, ps):
        for pr in range(2):
            vw = (gather(4 + pr, off) & rows(vmask[pr], WS)) | rows(vones[pr], WS)
            vbd = jnp.concatenate([pltpu.bitcast(vw, BF16), zpad], axis=0)
            o = _dot(ps[pr], vbd)
            for i in range(WS):
                os_ref[i, pr, pl.ds(off, 8), :] = o[8 * i:8 * i + 8, :]

    n_win = width // WS

    def attention_fast():
        pend = [scores(WS * w, False) for w in range(SKEW)]
        g = 0
        for w in range(n_win):
            if w + SKEW < n_win:
                pend.append(scores(WS * (w + SKEW), False))
            attend(WS * w, pend.pop(0))
            if w % 6 == 2 and g < CW // 8:
                conv_group(g)
                g += 1
        assert g == CW // 8

    def attention_exact():
        def body(qi, ps):
            base = pl.multiple_of(qi * (8 * WS), 8)
            for u in range(8):
                nxt = scores(base + WS * (u + 1), True)
                attend(base + WS * u, ps)
                ps = nxt
            return ps
        n_it = (n_win - 1) // 8
        ps = lax.fori_loop(0, n_it, body, scores(0, True))
        for w in range(n_it * 8, n_win):
            nxt = scores(WS * (w + 1), True) if w + 1 < n_win else None
            attend(WS * w, ps)
            ps = nxt
        conv_only()

    def out_load(it):
        i, l0 = tile_pos(it)
        ob = []
        for pr in range(2):
            o = os_ref[i, pr, pl.ds(l0, 128), :]
            den = jnp.take_along_axis(o, rows(den_idx[pr], 16), axis=1, mode="promise_in_bounds")
            ob.append((o * pltpu.reciprocal(den, approx=APPROX, full_range=False)).astype(BF16))
        return ob, res_ref[i, :, pl.ds(l0, 128)]

    def out_tile(it, pre=None):
        i, l0 = tile_pos(it)
        (oa, ob), rw = out_load(it) if pre is None else pre
        wa = pltpu.bitcast(wot_ref[:, 0:128], BF16)
        wb = pltpu.bitcast(wot_ref[:, 128:256], BF16)
        y = _dot(wa, oa, NT_DIMS) + _dot(wb, ob, NT_DIMS)
        ye = y[0:CW] + _lo(rw)
        yo = y[CW:C] + _hi(rw)
        o_ref[i, :, pl.ds(l0, 128)] = pltpu.bitcast(_pack2(ye, yo), BF16)

    def conv_only():
        def body(g, c):
            conv_group(g)
            return c
        lax.fori_loop(0, CW // 8, body, 0)

    def out_only():
        def body(it, c):
            out_tile(it)
            return c
        lax.fori_loop(0, NTILE, body, 0)

    def phase_b():
        for it in range(-LEAD, NTILE):
            if it + LEAD < NTILE:
                out_tile(it + LEAD)
                ln_tile(it + LEAD)
            if it >= 0:
                qkv_tile(it)

    @pl.when(s == 0)
    def _():
        _prepare_weights(dw_ref, wqkv_ref, wo_ref, dwt_ref, wq_ref, wot_ref)
        wq = pltpu.bitcast(wq_ref[...], BF16).astype(F32)
        sq = jnp.sum(wq * wq, axis=0, keepdims=True)
        l640 = _iota((1, 640), 1)
        t640, l128 = l640 >> 7, l640 & 127

        def norm2(tile, lo, hi):
            return jnp.sum(jnp.where((t640 == tile) & (l128 >= lo) & (l128 < hi), sq, 0.0))
        heads = [(0, 2, 0, 48), (0, 2, 48, 96), (1, 3, 32, 80), (1, 3, 80, 128)]
        bound2 = 0.0
        for tq, tk, lo, hi in heads:
            bound2 = jnp.maximum(bound2, norm2(tq, lo, hi) * norm2(tk, lo, hi))
        safe = bound2 * (1.1 * C * c_exp) ** 2 <= EXP_LIMIT ** 2
        flag_ref[0] = jnp.where(safe, 1, 0).astype(jnp.int32)
        os_ref[...] = jnp.ones(os_ref.shape, F32)
        res_ref[...] = jnp.zeros(res_ref.shape, U32)
        conv_only()

    @pl.when((s > 0) & (s <= n_strips))
    def _():
        phase_b()
        safe = flag_ref[0] == 1

        @pl.when(safe)
        def _():
            attention_fast()

        @pl.when(jnp.logical_not(safe))
        def _():
            attention_exact()

    @pl.when(s == n_strips + 1)
    def _():
        out_only()


@jax.jit
def pallas_standalone__window_attn_davit__vision_kernel(
    x: jax.Array,
    dw_pe: jax.Array,
    w_qkv: jax.Array,
    w_o: jax.Array,
):
    B, H, W, Cc = x.shape
    assert B == 1 and Cc == C and dw_pe.shape == (3, 3, C)
    assert H % WS == 0 and W % WS == 0 and 384 < W <= 512
    n_strips = H // WS
    xt = jnp.transpose(x, (0, 1, 3, 2)).reshape(H, C, W)
    dw = dw_pe.reshape(9, C)

    strip = lambda a: jnp.minimum(a, n_strips - 1)
    full = lambda shape: pl.BlockSpec(shape, lambda a: (0,) * len(shape))
    out = pl.pallas_call(
        functools.partial(_kernel, n_strips=n_strips, width=W),
        grid=(n_strips + 2,),
        in_specs=[
            pl.BlockSpec((WS, C, 512), lambda a: (strip(a), 0, 0)),
            pl.BlockSpec((1, C, 512), lambda a: (jnp.maximum(strip(a) * WS - 1, 0), 0, 0)),
            pl.BlockSpec((1, C, 512), lambda a: (jnp.minimum(strip(a) * WS + WS, H - 1), 0, 0)),
            full((9, C)),
            full((C, 3 * C)),
            full((C, C)),
        ],
        out_specs=pl.BlockSpec((WS, C, 512), lambda a: (jnp.maximum(a - 2, 0), 0, 0)),
        out_shape=jax.ShapeDtypeStruct((H, C, W), x.dtype),
        scratch_shapes=[
            pltpu.VMEM((9, 2, CW, 128), F32),
            pltpu.VMEM((128, 640), U32),
            pltpu.VMEM((CW, 256), U32),
            pltpu.VMEM((WS, 2, CW, 512), F32),
            pltpu.VMEM((WS, CW, 512), U32),
            pltpu.VMEM((WS, 512, 128), U32),
            pltpu.VMEM((WS, 6, 512, 128), U32),
            pltpu.VMEM((WS, 2, 512, 128), F32),
            pltpu.SMEM((1,), jnp.int32),
        ],
        compiler_params=pltpu.CompilerParams(
            dimension_semantics=("arbitrary",),
            vmem_limit_bytes=100 * 1024 * 1024,
        ),
    )(xt, xt, xt, dw, w_qkv, w_o)
    return jnp.transpose(out.reshape(B, H, C, W), (0, 1, 3, 2))
```

```python
import functools

import jax
import jax.numpy as jnp
import jax.experimental.pallas as pl
import jax.experimental.pallas.tpu as pltpu
from jax import lax

WS = 7
NH = 4
C = 192
DH = C // NH
CW = C // 2
F32 = jnp.float32
BF16 = jnp.bfloat16
U32 = jnp.uint32
NT_DIMS = (((1,), (1,)), ((), ()))
NN_DIMS = (((1,), (0,)), ((), ()))
NEG = -1e30
LOG2E = 1.4426950408889634
UW = 8
SKEW = 1
LEAD = 2
QORDER = (0, 1, 2, 3, 4)
XLEAD = 2
OLEAD = 2
QORDER = (0, 1, 2, 3, 4)
OPRE = 0
EXP_LIMIT = 40.0
UC = 2
APPROX = True


def _dot(a, b, dims=NN_DIMS):
    return lax.dot_general(a, b, dims, preferred_element_type=F32)


def _iota(shape, dim):
    return lax.broadcasted_iota(jnp.int32, shape, dim)


def _f32(words):
    return pltpu.bitcast(words, F32)


def _lo(words):
    return _f32(words << 16)


def _hi(words):
    return _f32(words & U32(0xFFFF0000))


def _pack2(a, b):
    return pltpu.pack_elementwise([a, b], packed_dtype=BF16)


def _onehot(rows_map, cols_map):
    return jnp.where(rows_map == cols_map, 1.0, 0.0).astype(BF16)


def _prepare_weights(dw_ref, wqkv_ref, wo_ref, dwt_ref, wq_ref, wot_ref):
    r_i = _iota((CW, C), 0)
    c_i = _iota((CW, C), 1)
    for p in range(2):
        sel = _onehot(2 * r_i + p, c_i)
        for k in range(9):
            rep = jnp.broadcast_to(dw_ref[k:k + 1, :], (128, C))
            t = _dot(sel, rep, NT_DIMS)
            if k == 4:
                t = t + 1.0
            dwt_ref[k, p] = t
    rho = _iota((256, C), 0)
    rr = rho & 127
    chan = jnp.where(rr < CW, 2 * rr + (rho >> 7), -1)
    rsel = _onehot(chan, _iota((256, C), 1))
    w1 = _dot(rsel, wqkv_ref[...]).astype(BF16)
    n = _iota((3 * C, 640), 1)
    l = n & 127
    t = n >> 7
    col0 = jnp.where(l < 96, l, 384 + 64 + l - 96)
    col1 = jnp.where(l >= 32, 96 + l - 32, 384 + l)
    col2 = jnp.where(l < 96, 192 + l, -1)
    col3 = jnp.where(l >= 32, 288 + l - 32, -1)
    col4 = jnp.where(l < 32, 480 + l, jnp.where(l < 64, 384 + l, 448 + l))
    col = jnp.where(t == 0, col0, jnp.where(t == 1, col1, jnp.where(t == 2, col2,
                    jnp.where(t == 3, col3, col4))))
    csel = _onehot(_iota((3 * C, 640), 0), col)
    wq = _dot(w1, csel)
    wq_ref[...] = pltpu.bitcast(wq.astype(BF16), U32)
    lam = _iota((256, C), 0)
    ll = lam & 127
    fa = jnp.where(ll < 64, ll, jnp.where(ll < 96, -1, ll - 32))
    fb = jnp.where(ll < 32, 96 + ll, jnp.where(ll < 64, -1, 64 + ll))
    feat = jnp.where(lam < 128, fa, fb)
    fsel = _onehot(feat, _iota((256, C), 1))
    tmp = _dot(fsel, wo_ref[...]).astype(BF16)
    rp = _iota((C, C), 0)
    ochan = jnp.where(rp < CW, 2 * rp, 2 * (rp - CW) + 1)
    osel = _onehot(ochan, _iota((C, C), 1))
    wot_ref[...] = pltpu.bitcast(_dot(osel, tmp, NT_DIMS).astype(BF16), U32)


def _kernel(xm_ref, xt_ref, xb_ref, dw_ref, wqkv_ref, wo_ref, o_ref,
            dwt_ref, wq_ref, wot_ref, x0_ref, res_ref, hs_ref, qkv_ref, os_ref, flag_ref,
            *, n_strips, width):
    s = pl.program_id(0)
    WP = 512
    NTILE = WS * 4

    sub = _iota((8, 128), 0)
    lane = _iota((8, 128), 1)
    lo16, hi16 = U32(0x0000FFFF), U32(0xFFFF0000)
    zero = U32(0)

    def rows(m, n):
        return jnp.concatenate([m] * n, axis=0)

    def halves(hp0, hp1):
        return jnp.where(hp0, lo16, jnp.where(hp1, hi16, zero))

    key_ok = sub < WS
    kmask = [halves(lane < 48, (lane >= 48) & (lane < 96)),
             halves((lane >= 32) & (lane < 80), lane >= 80)]
    va1 = ((lane >= 48) & (lane < 64)) | (lane >= 96)
    vb1 = lane >= 80
    vmask = [halves(lane < 48, va1), halves((lane < 32) | ((lane >= 64) & (lane < 80)), vb1)]
    key_mask = jnp.where(key_ok, U32(0xFFFFFFFF), zero)
    one_lo, one_hi = U32(0x00003F80), U32(0x3F800000)

    def ones(d0):
        m = jnp.where((lane >= d0) & (lane < d0 + 16), one_lo,
                      jnp.where((lane >= d0 + 16) & (lane < d0 + 32), one_hi, zero))
        return m

    vones = [ones(64), ones(32)]
    den_idx = [jnp.where(va1, 80, 64), jnp.where(vb1, 48, 32)]
    even = (lane & 1) == 0
    s_valid = ((lane & 15) < 14) & (lane < 112)
    quarter = lane >> 5
    last_valid = lane < (width - 384)
    c_exp = (DH ** -0.5) * LOG2E

    def conv_steps(g):
        top_ok = s > 0
        bot_ok = s < n_strips - 1
        c0 = g * 16 if isinstance(g, int) else pl.multiple_of(g * 16, 16)
        r0 = g * 8 if isinstance(g, int) else pl.multiple_of(g * 8, 8)
        taps = [[jnp.concatenate([dwt_ref[k, p, pl.ds(r0, 8), :]] * 4, axis=1)
                 for p in range(2)] for k in range(9)]
        acc = {}
        for r in range(-1, WS + 1):
            if r == -1:
                raw = xt_ref[0, pl.ds(c0, 16), :]
            elif r == WS:
                raw = xb_ref[0, pl.ds(c0, 16), :]
            else:
                raw = xm_ref[r, pl.ds(c0, 16), :]
            w = pltpu.bitcast(raw, U32)
            w = jnp.concatenate([w[:, :384], jnp.where(last_valid, w[:, 384:], zero)], axis=1)
            if r == -1:
                w = jnp.where(top_ok, w, zero)
            if r == WS:
                w = jnp.where(bot_ok, w, zero)
            sh = [pltpu.roll(w, 1, 1), w, pltpu.roll(w, WP - 1, 1)]
            for p, unp in enumerate((_lo, _hi)):
                u = [unp(t) for t in sh]
                for i in range(3):
                    orow = r + 1 - i
                    if orow < 0 or orow >= WS:
                        continue
                    t = u[0] * taps[3 * i][p] + u[1] * taps[3 * i + 1][p] + u[2] * taps[3 * i + 2][p]
                    key = (orow, p)
                    acc[key] = t if key not in acc else acc[key] + t
                    if i == 2:
                        x0_ref[orow, p, pl.ds(r0, 8), :] = acc.pop(key)
            yield

    def conv_group(g):
        for _ in conv_steps(g):
            pass

    def tile_pos(it):
        if isinstance(it, int):
            return it // 4, (it % 4) * 128
        return it >> 2, pl.multiple_of((it & 3) * 128, 128)

    def ln_tile(it):
        i, l0 = tile_pos(it)
        xe = x0_ref[i, 0, :, pl.ds(l0, 128)]
        xo = x0_ref[i, 1, :, pl.ds(l0, 128)]
        res_ref[i, :, pl.ds(l0, 128)] = _pack2(xe, xo)
        mean = jnp.sum(xe + xo, axis=0, keepdims=True) * (1.0 / C)
        de = xe - mean
        do = xo - mean
        var = jnp.sum(de * de + do * do, axis=0, keepdims=True) * (1.0 / C)
        rstd = lax.rsqrt(var + 1e-5)
        return _pack2(de * rstd, do * rstd)

    def xpose_tile(it, words):
        i, l0 = tile_pos(it)
        words = jnp.concatenate([words, jnp.zeros((128 - CW, 128), U32)], axis=0)
        words = words.T
        t0 = l0 // 2 if isinstance(l0, int) else pl.multiple_of(l0 >> 1, 64)
        for p, unp in enumerate((_lo, _hi)):
            hs_ref[i, p, pl.ds(t0, 64), :] = pltpu.bitcast(unp(words).astype(BF16), U32)

    def qkv_tile(it):
        i, l0 = tile_pos(it)
        t0 = l0 // 2 if isinstance(l0, int) else pl.multiple_of(l0 >> 1, 64)
        he = pltpu.bitcast(hs_ref[i, 0, pl.ds(t0, 64), :], BF16)
        ho = pltpu.bitcast(hs_ref[i, 1, pl.ds(t0, 64), :], BF16)
        q16 = rows(quarter, 16)
        dst = lambda j: qkv_ref.at[i, j, pl.ds(l0, 128), :]
        for j in QORDER:
            we = pltpu.bitcast(wq_ref[0:64, 128 * j:128 * (j + 1)], BF16)
            wo = pltpu.bitcast(wq_ref[64:128, 128 * j:128 * (j + 1)], BF16)
            t = _dot(he, we) + _dot(ho, wo)
            if j == 4:
                w = _pack2(t, t)
                dst(5)[...] = (w & rows(vmask[1], 16)) | rows(vones[1], 16)
                pltpu.store(dst(4), w & rows(vmask[0], 16), mask=q16 == 1)
                pltpu.store(dst(4), rows(vones[0], 16), mask=q16 == 2)
            elif j < 2:
                dst(j)[...] = pltpu.bitcast(t * c_exp, U32)
                pltpu.store(dst(4), _pack2(t, t) & rows(vmask[0], 16), mask=q16 == (3 if j == 0 else 0))
            else:
                dst(j)[...] = _pack2(t, t) & rows(kmask[j - 2], 16)

    zpad = jnp.zeros((16, 128), BF16)

    def gather(j, off):
        return jnp.concatenate([qkv_ref[i, j, pl.ds(off, 8), :] for i in range(WS)], axis=0)

    def scores(off, exact_max):
        ps = []
        for pr in range(2):
            q = _f32(gather(pr, off))
            kbd = jnp.concatenate([pltpu.bitcast(gather(2 + pr, off), BF16), zpad], axis=0)
            sc = _dot(q, kbd, NT_DIMS)
            if exact_max:
                sc = jnp.where(rows(s_valid, WS), sc, NEG)
                ev = rows(even, WS)
                m0 = jnp.max(jnp.where(ev, sc, NEG), axis=1, keepdims=True)
                m1 = jnp.max(jnp.where(ev, NEG, sc), axis=1, keepdims=True)
                sc = sc - jnp.where(ev, m0, m1)
            ps.append(jnp.exp2(sc))
        return ps

    def attend(off, ps):
        for pr in range(2):
            vw = gather(4 + pr, off) & rows(key_mask, WS)
            vbd = jnp.concatenate([pltpu.bitcast(vw, BF16), zpad], axis=0)
            o = _dot(ps[pr], vbd)
            for i in range(WS):
                os_ref[i, pr, pl.ds(off, 8), :] = o[8 * i:8 * i + 8, :]

    n_win = width // WS

    def attention_fast():
        steps = (None for gg in range(CW // 8) for _ in conv_steps(gg))
        n_steps = (CW // 8) * (WS + 2)
        pend = [scores(WS * w, False) for w in range(SKEW)]
        g = 0
        for w in range(n_win):
            if w + SKEW < n_win:
                pend.append(scores(WS * (w + SKEW), False))
            attend(WS * w, pend.pop(0))
            while g * n_win < (w + 1) * n_steps:
                next(steps, None)
                g += 1
        for _ in steps:
            pass

    def attention_exact():
        def body(qi, ps):
            base = pl.multiple_of(qi * (8 * WS), 8)
            for u in range(8):
                nxt = scores(base + WS * (u + 1), True)
                attend(base + WS * u, ps)
                ps = nxt
            return ps
        n_it = (n_win - 1) // 8
        ps = lax.fori_loop(0, n_it, body, scores(0, True))
        for w in range(n_it * 8, n_win):
            nxt = scores(WS * (w + 1), True) if w + 1 < n_win else None
            attend(WS * w, ps)
            ps = nxt
        conv_only()

    def out_load(it):
        i, l0 = tile_pos(it)
        ob = []
        for pr in range(2):
            o = os_ref[i, pr, pl.ds(l0, 128), :]
            den = jnp.take_along_axis(o, rows(den_idx[pr], 16), axis=1, mode="promise_in_bounds")
            ob.append((o * pltpu.reciprocal(den, approx=APPROX, full_range=False)).astype(BF16))
        return ob, res_ref[i, :, pl.ds(l0, 128)]

    def out_tile(it, pre=None):
        i, l0 = tile_pos(it)
        (oa, ob), rw = out_load(it) if pre is None else pre
        wa = pltpu.bitcast(wot_ref[:, 0:128], BF16)
        wb = pltpu.bitcast(wot_ref[:, 128:256], BF16)
        y = _dot(wa, oa, NT_DIMS) + _dot(wb, ob, NT_DIMS)
        ye = y[0:CW] + _lo(rw)
        yo = y[CW:C] + _hi(rw)
        o_ref[i, :, pl.ds(l0, 128)] = pltpu.bitcast(_pack2(ye, yo), BF16)

    def conv_only():
        def body(g, c):
            conv_group(g)
            return c
        lax.fori_loop(0, CW // 8, body, 0)

    def out_only():
        def body(it, c):
            out_tile(it)
            return c
        lax.fori_loop(0, NTILE, body, 0)

    def phase_b():
        words, pre = {}, {}
        for it in range(-LEAD, NTILE):
            t = it + OLEAD + OPRE
            if 0 <= t < NTILE:
                pre[t] = out_load(t)
            t = it + OLEAD
            if 0 <= t < NTILE:
                out_tile(t, pre.pop(t))
            t = it + LEAD
            if 0 <= t < NTILE:
                words[t] = ln_tile(t)
            t = it + XLEAD
            if 0 <= t < NTILE:
                xpose_tile(t, words.pop(t))
            if it >= 0:
                qkv_tile(it)

    @pl.when(s == 0)
    def _():
        _prepare_weights(dw_ref, wqkv_ref, wo_ref, dwt_ref, wq_ref, wot_ref)
        wq = pltpu.bitcast(wq_ref[...], BF16).astype(F32)
        sq = jnp.sum(wq * wq, axis=0, keepdims=True)
        l640 = _iota((1, 640), 1)
        t640, l128 = l640 >> 7, l640 & 127

        def norm2(tile, lo, hi):
            return jnp.sum(jnp.where((t640 == tile) & (l128 >= lo) & (l128 < hi), sq, 0.0))
        heads = [(0, 2, 0, 48), (0, 2, 48, 96), (1, 3, 32, 80), (1, 3, 80, 128)]
        bound2 = 0.0
        for tq, tk, lo, hi in heads:
            bound2 = jnp.maximum(bound2, norm2(tq, lo, hi) * norm2(tk, lo, hi))
        safe = bound2 * (1.1 * C * c_exp) ** 2 <= EXP_LIMIT ** 2
        flag_ref[0] = jnp.where(safe, 1, 0).astype(jnp.int32)
        os_ref[...] = jnp.ones(os_ref.shape, F32)
        res_ref[...] = jnp.zeros(res_ref.shape, U32)
        conv_only()

    @pl.when((s > 0) & (s <= n_strips))
    def _():
        phase_b()
        safe = flag_ref[0] == 1

        @pl.when(safe)
        def _():
            attention_fast()

        @pl.when(jnp.logical_not(safe))
        def _():
            attention_exact()

    @pl.when(s == n_strips + 1)
    def _():
        out_only()


@jax.jit
def pallas_standalone__window_attn_davit__vision_kernel(
    x: jax.Array,
    dw_pe: jax.Array,
    w_qkv: jax.Array,
    w_o: jax.Array,
):
    B, H, W, Cc = x.shape
    assert B == 1 and Cc == C and dw_pe.shape == (3, 3, C)
    assert H % WS == 0 and W % WS == 0 and 384 < W <= 512
    n_strips = H // WS
    xt = jnp.transpose(x, (0, 1, 3, 2)).reshape(H, C, W)
    dw = dw_pe.reshape(9, C)

    strip = lambda a: jnp.minimum(a, n_strips - 1)
    full = lambda shape: pl.BlockSpec(shape, lambda a: (0,) * len(shape))
    out = pl.pallas_call(
        functools.partial(_kernel, n_strips=n_strips, width=W),
        grid=(n_strips + 2,),
        in_specs=[
            pl.BlockSpec((WS, C, 512), lambda a: (strip(a), 0, 0)),
            pl.BlockSpec((1, C, 512), lambda a: (jnp.maximum(strip(a) * WS - 1, 0), 0, 0)),
            pl.BlockSpec((1, C, 512), lambda a: (jnp.minimum(strip(a) * WS + WS, H - 1), 0, 0)),
            full((9, C)),
            full((C, 3 * C)),
            full((C, C)),
        ],
        out_specs=pl.BlockSpec((WS, C, 512), lambda a: (jnp.maximum(a - 2, 0), 0, 0)),
        out_shape=jax.ShapeDtypeStruct((H, C, W), x.dtype),
        scratch_shapes=[
            pltpu.VMEM((9, 2, CW, 128), F32),
            pltpu.VMEM((128, 640), U32),
            pltpu.VMEM((CW, 256), U32),
            pltpu.VMEM((WS, 2, CW, 512), F32),
            pltpu.VMEM((WS, CW, 512), U32),
            pltpu.VMEM((WS, 2, 256, 128), U32),
            pltpu.VMEM((WS, 6, 512, 128), U32),
            pltpu.VMEM((WS, 2, 512, 128), F32),
            pltpu.SMEM((1,), jnp.int32),
        ],
        compiler_params=pltpu.CompilerParams(
            dimension_semantics=("arbitrary",),
            vmem_limit_bytes=100 * 1024 * 1024,
        ),
    )(xt, xt, xt, dw, w_qkv, w_o)
    return jnp.transpose(out.reshape(B, H, C, W), (0, 1, 3, 2))
```

```python
import functools

import jax
import jax.numpy as jnp
import jax.experimental.pallas as pl
import jax.experimental.pallas.tpu as pltpu
from jax import lax

WS = 7
NH = 4
C = 192
DH = C // NH
CW = C // 2
F32 = jnp.float32
BF16 = jnp.bfloat16
U32 = jnp.uint32
NT_DIMS = (((1,), (1,)), ((), ()))
NN_DIMS = (((1,), (0,)), ((), ()))
NEG = -1e30
LOG2E = 1.4426950408889634
UW = 8
SKEW = 1
LEAD = 2
PSPLIT = 1
QORDER = (0, 1, 2, 3, 4)
XLEAD = 2
PSPLIT = 1
OLEAD = 2
PSPLIT = 1
QORDER = (0, 1, 2, 3, 4)
OPRE = 0
EXP_LIMIT = 40.0
UC = 2
APPROX = True


def _dot(a, b, dims=NN_DIMS):
    return lax.dot_general(a, b, dims, preferred_element_type=F32)


def _iota(shape, dim):
    return lax.broadcasted_iota(jnp.int32, shape, dim)


def _f32(words):
    return pltpu.bitcast(words, F32)


def _lo(words):
    return _f32(words << 16)


def _hi(words):
    return _f32(words & U32(0xFFFF0000))


def _pack2(a, b):
    return pltpu.pack_elementwise([a, b], packed_dtype=BF16)


def _onehot(rows_map, cols_map):
    return jnp.where(rows_map == cols_map, 1.0, 0.0).astype(BF16)


def _prepare_weights(dw_ref, wqkv_ref, wo_ref, dwt_ref, wq_ref, wot_ref):
    r_i = _iota((CW, C), 0)
    c_i = _iota((CW, C), 1)
    for p in range(2):
        sel = _onehot(2 * r_i + p, c_i)
        for k in range(9):
            rep = jnp.broadcast_to(dw_ref[k:k + 1, :], (128, C))
            t = _dot(sel, rep, NT_DIMS)
            if k == 4:
                t = t + 1.0
            dwt_ref[k, p] = t
    rho = _iota((256, C), 0)
    rr = rho & 127
    chan = jnp.where(rr < CW, 2 * rr + (rho >> 7), -1)
    rsel = _onehot(chan, _iota((256, C), 1))
    w1 = _dot(rsel, wqkv_ref[...]).astype(BF16)
    n = _iota((3 * C, 640), 1)
    l = n & 127
    t = n >> 7
    col0 = jnp.where(l < 96, l, 384 + 64 + l - 96)
    col1 = jnp.where(l >= 32, 96 + l - 32, 384 + l)
    col2 = jnp.where(l < 96, 192 + l, -1)
    col3 = jnp.where(l >= 32, 288 + l - 32, -1)
    col4 = jnp.where(l < 32, 480 + l, jnp.where(l < 64, 384 + l, 448 + l))
    col = jnp.where(t == 0, col0, jnp.where(t == 1, col1, jnp.where(t == 2, col2,
                    jnp.where(t == 3, col3, col4))))
    csel = _onehot(_iota((3 * C, 640), 0), col)
    wq = _dot(w1, csel)
    wq_ref[...] = pltpu.bitcast(wq.astype(BF16), U32)
    lam = _iota((256, C), 0)
    ll = lam & 127
    fa = jnp.where(ll < 64, ll, jnp.where(ll < 96, -1, ll - 32))
    fb = jnp.where(ll < 32, 96 + ll, jnp.where(ll < 64, -1, 64 + ll))
    feat = jnp.where(lam < 128, fa, fb)
    fsel = _onehot(feat, _iota((256, C), 1))
    tmp = _dot(fsel, wo_ref[...]).astype(BF16)
    rp = _iota((C, C), 0)
    ochan = jnp.where(rp < CW, 2 * rp, 2 * (rp - CW) + 1)
    osel = _onehot(ochan, _iota((C, C), 1))
    wot_ref[...] = pltpu.bitcast(_dot(osel, tmp, NT_DIMS).astype(BF16), U32)


def _kernel(xm_ref, xt_ref, xb_ref, dw_ref, wqkv_ref, wo_ref, o_ref,
            dwt_ref, wq_ref, wot_ref, x0_ref, res_ref, hs_ref, qkv_ref, os_ref, flag_ref,
            *, n_strips, width):
    s = pl.program_id(0)
    WP = 512
    NTILE = WS * 4

    sub = _iota((8, 128), 0)
    lane = _iota((8, 128), 1)
    lo16, hi16 = U32(0x0000FFFF), U32(0xFFFF0000)
    zero = U32(0)

    def rows(m, n):
        return jnp.concatenate([m] * n, axis=0)

    def halves(hp0, hp1):
        return jnp.where(hp0, lo16, jnp.where(hp1, hi16, zero))

    key_ok = sub < WS
    kmask = [halves(lane < 48, (lane >= 48) & (lane < 96)),
             halves((lane >= 32) & (lane < 80), lane >= 80)]
    va1 = ((lane >= 48) & (lane < 64)) | (lane >= 96)
    vb1 = lane >= 80
    vmask = [halves(lane < 48, va1), halves((lane < 32) | ((lane >= 64) & (lane < 80)), vb1)]
    key_mask = jnp.where(key_ok, U32(0xFFFFFFFF), zero)
    one_lo, one_hi = U32(0x00003F80), U32(0x3F800000)

    def ones(d0):
        m = jnp.where((lane >= d0) & (lane < d0 + 16), one_lo,
                      jnp.where((lane >= d0 + 16) & (lane < d0 + 32), one_hi, zero))
        return m

    vones = [ones(64), ones(32)]
    den_idx = [jnp.where(va1, 80, 64), jnp.where(vb1, 48, 32)]
    even = (lane & 1) == 0
    s_valid = ((lane & 15) < 14) & (lane < 112)
    quarter = lane >> 5
    last_valid = lane < (width - 384)
    c_exp = (DH ** -0.5) * LOG2E

    def conv_steps(g):
        top_ok = s > 0
        bot_ok = s < n_strips - 1
        c0 = g * 16 if isinstance(g, int) else pl.multiple_of(g * 16, 16)
        r0 = g * 8 if isinstance(g, int) else pl.multiple_of(g * 8, 8)
        for p, unp in enumerate((_lo, _hi)):
            taps = [jnp.concatenate([dwt_ref[k, p, pl.ds(r0, 8), :]] * 4, axis=1) for k in range(9)]
            xs = {}
            for r in range(-1, WS + 1):
                if r == -1:
                    raw = xt_ref[0, pl.ds(c0, 16), :]
                elif r == WS:
                    raw = xb_ref[0, pl.ds(c0, 16), :]
                else:
                    raw = xm_ref[r, pl.ds(c0, 16), :]
                w = pltpu.bitcast(raw, U32)
                w = jnp.concatenate([w[:, :384], jnp.where(last_valid, w[:, 384:], zero)], axis=1)
                if r == -1:
                    w = jnp.where(top_ok, w, zero)
                if r == WS:
                    w = jnp.where(bot_ok, w, zero)
                xs[r] = unp(w)
                if r >= 1:
                    i = r - 1
                    t = [xs[i - 1] * taps[j] + xs[i] * taps[3 + j] + xs[i + 1] * taps[6 + j]
                         for j in range(3)]
                    x0_ref[i, p, pl.ds(r0, 8), :] = (
                        pltpu.roll(t[0], 1, 1) + t[1] + pltpu.roll(t[2], WP - 1, 1))
                    del xs[i - 1]
                if p == 1 or not PSPLIT:
                    yield

    def conv_group(g):
        for _ in conv_steps(g):
            pass

    def tile_pos(it):
        if isinstance(it, int):
            return it // 4, (it % 4) * 128
        return it >> 2, pl.multiple_of((it & 3) * 128, 128)

    def ln_tile(it):
        i, l0 = tile_pos(it)
        xe = x0_ref[i, 0, :, pl.ds(l0, 128)]
        xo = x0_ref[i, 1, :, pl.ds(l0, 128)]
        res_ref[i, :, pl.ds(l0, 128)] = _pack2(xe, xo)
        mean = jnp.sum(xe + xo, axis=0, keepdims=True) * (1.0 / C)
        de = xe - mean
        do = xo - mean
        var = jnp.sum(de * de + do * do, axis=0, keepdims=True) * (1.0 / C)
        rstd = lax.rsqrt(var + 1e-5)
        return _pack2(de * rstd, do * rstd)

    def xpose_tile(it, words):
        i, l0 = tile_pos(it)
        words = jnp.concatenate([words, jnp.zeros((128 - CW, 128), U32)], axis=0)
        words = words.T
        t0 = l0 // 2 if isinstance(l0, int) else pl.multiple_of(l0 >> 1, 64)
        for p, unp in enumerate((_lo, _hi)):
            hs_ref[i, p, pl.ds(t0, 64), :] = pltpu.bitcast(unp(words).astype(BF16), U32)

    def qkv_tile(it):
        i, l0 = tile_pos(it)
        t0 = l0 // 2 if isinstance(l0, int) else pl.multiple_of(l0 >> 1, 64)
        he = pltpu.bitcast(hs_ref[i, 0, pl.ds(t0, 64), :], BF16)
        ho = pltpu.bitcast(hs_ref[i, 1, pl.ds(t0, 64), :], BF16)
        q16 = rows(quarter, 16)
        dst = lambda j: qkv_ref.at[i, j, pl.ds(l0, 128), :]
        for j in QORDER:
            we = pltpu.bitcast(wq_ref[0:64, 128 * j:128 * (j + 1)], BF16)
            wo = pltpu.bitcast(wq_ref[64:128, 128 * j:128 * (j + 1)], BF16)
            t = _dot(he, we) + _dot(ho, wo)
            if j == 4:
                w = _pack2(t, t)
                dst(5)[...] = (w & rows(vmask[1], 16)) | rows(vones[1], 16)
                pltpu.store(dst(4), w & rows(vmask[0], 16), mask=q16 == 1)
                pltpu.store(dst(4), rows(vones[0], 16), mask=q16 == 2)
            elif j < 2:
                dst(j)[...] = pltpu.bitcast(t * c_exp, U32)
                pltpu.store(dst(4), _pack2(t, t) & rows(vmask[0], 16), mask=q16 == (3 if j == 0 else 0))
            else:
                dst(j)[...] = _pack2(t, t) & rows(kmask[j - 2], 16)

    zpad = jnp.zeros((16, 128), BF16)

    def gather(j, off):
        return jnp.concatenate([qkv_ref[i, j, pl.ds(off, 8), :] for i in range(WS)], axis=0)

    def scores(off, exact_max):
        ps = []
        for pr in range(2):
            q = _f32(gather(pr, off))
            kbd = jnp.concatenate([pltpu.bitcast(gather(2 + pr, off), BF16), zpad], axis=0)
            sc = _dot(q, kbd, NT_DIMS)
            if exact_max:
                sc = jnp.where(rows(s_valid, WS), sc, NEG)
                ev = rows(even, WS)
                m0 = jnp.max(jnp.where(ev, sc, NEG), axis=1, keepdims=True)
                m1 = jnp.max(jnp.where(ev, NEG, sc), axis=1, keepdims=True)
                sc = sc - jnp.where(ev, m0, m1)
            ps.append(jnp.exp2(sc))
        return ps

    def attend(off, ps):
        for pr in range(2):
            vw = gather(4 + pr, off) & rows(key_mask, WS)
            vbd = jnp.concatenate([pltpu.bitcast(vw, BF16), zpad], axis=0)
            o = _dot(ps[pr], vbd)
            for i in range(WS):
                os_ref[i, pr, pl.ds(off, 8), :] = o[8 * i:8 * i + 8, :]

    n_win = width // WS

    def attention_fast():
        steps = (None for gg in range(CW // 8) for _ in conv_steps(gg))
        n_steps = (CW // 8) * (WS + 2)
        pend = [scores(WS * w, False) for w in range(SKEW)]
        g = 0
        for w in range(n_win):
            if w + SKEW < n_win:
                pend.append(scores(WS * (w + SKEW), False))
            attend(WS * w, pend.pop(0))
            while g * n_win < (w + 1) * n_steps:
                next(steps, None)
                g += 1
        for _ in steps:
            pass

    def attention_exact():
        def body(qi, ps):
            base = pl.multiple_of(qi * (8 * WS), 8)
            for u in range(8):
                nxt = scores(base + WS * (u + 1), True)
                attend(base + WS * u, ps)
                ps = nxt
            return ps
        n_it = (n_win - 1) // 8
        ps = lax.fori_loop(0, n_it, body, scores(0, True))
        for w in range(n_it * 8, n_win):
            nxt = scores(WS * (w + 1), True) if w + 1 < n_win else None
            attend(WS * w, ps)
            ps = nxt
        conv_only()

    def out_load(it):
        i, l0 = tile_pos(it)
        ob = []
        for pr in range(2):
            o = os_ref[i, pr, pl.ds(l0, 128), :]
            den = jnp.take_along_axis(o, rows(den_idx[pr], 16), axis=1, mode="promise_in_bounds")
            ob.append((o * pltpu.reciprocal(den, approx=APPROX, full_range=False)).astype(BF16))
        return ob, res_ref[i, :, pl.ds(l0, 128)]

    def out_tile(it, pre=None):
        i, l0 = tile_pos(it)
        (oa, ob), rw = out_load(it) if pre is None else pre
        wa = pltpu.bitcast(wot_ref[:, 0:128], BF16)
        wb = pltpu.bitcast(wot_ref[:, 128:256], BF16)
        y = _dot(wa, oa, NT_DIMS) + _dot(wb, ob, NT_DIMS)
        ye = y[0:CW] + _lo(rw)
        yo = y[CW:C] + _hi(rw)
        o_ref[i, :, pl.ds(l0, 128)] = pltpu.bitcast(_pack2(ye, yo), BF16)

    def conv_only():
        def body(g, c):
            conv_group(g)
            return c
        lax.fori_loop(0, CW // 8, body, 0)

    def out_only():
        def body(it, c):
            out_tile(it)
            return c
        lax.fori_loop(0, NTILE, body, 0)

    def phase_b():
        words, pre = {}, {}
        for it in range(-LEAD, NTILE):
            t = it + OLEAD + OPRE
            if 0 <= t < NTILE:
                pre[t] = out_load(t)
            t = it + OLEAD
            if 0 <= t < NTILE:
                out_tile(t, pre.pop(t))
            t = it + LEAD
            if 0 <= t < NTILE:
                words[t] = ln_tile(t)
            t = it + XLEAD
            if 0 <= t < NTILE:
                xpose_tile(t, words.pop(t))
            if it >= 0:
                qkv_tile(it)

    @pl.when(s == 0)
    def _():
        _prepare_weights(dw_ref, wqkv_ref, wo_ref, dwt_ref, wq_ref, wot_ref)
        wq = pltpu.bitcast(wq_ref[...], BF16).astype(F32)
        sq = jnp.sum(wq * wq, axis=0, keepdims=True)
        l640 = _iota((1, 640), 1)
        t640, l128 = l640 >> 7, l640 & 127

        def norm2(tile, lo, hi):
            return jnp.sum(jnp.where((t640 == tile) & (l128 >= lo) & (l128 < hi), sq, 0.0))
        heads = [(0, 2, 0, 48), (0, 2, 48, 96), (1, 3, 32, 80), (1, 3, 80, 128)]
        bound2 = 0.0
        for tq, tk, lo, hi in heads:
            bound2 = jnp.maximum(bound2, norm2(tq, lo, hi) * norm2(tk, lo, hi))
        safe = bound2 * (1.1 * C * c_exp) ** 2 <= EXP_LIMIT ** 2
        flag_ref[0] = jnp.where(safe, 1, 0).astype(jnp.int32)
        os_ref[...] = jnp.ones(os_ref.shape, F32)
        res_ref[...] = jnp.zeros(res_ref.shape, U32)
        conv_only()

    @pl.when((s > 0) & (s <= n_strips))
    def _():
        phase_b()
        safe = flag_ref[0] == 1

        @pl.when(safe)
        def _():
            attention_fast()

        @pl.when(jnp.logical_not(safe))
        def _():
            attention_exact()

    @pl.when(s == n_strips + 1)
    def _():
        out_only()


@jax.jit
def pallas_standalone__window_attn_davit__vision_kernel(
    x: jax.Array,
    dw_pe: jax.Array,
    w_qkv: jax.Array,
    w_o: jax.Array,
):
    B, H, W, Cc = x.shape
    assert B == 1 and Cc == C and dw_pe.shape == (3, 3, C)
    assert H % WS == 0 and W % WS == 0 and 384 < W <= 512
    n_strips = H // WS
    xt = jnp.transpose(x, (0, 1, 3, 2)).reshape(H, C, W)
    dw = dw_pe.reshape(9, C)

    strip = lambda a: jnp.minimum(a, n_strips - 1)
    full = lambda shape: pl.BlockSpec(shape, lambda a: (0,) * len(shape))
    out = pl.pallas_call(
        functools.partial(_kernel, n_strips=n_strips, width=W),
        grid=(n_strips + 2,),
        in_specs=[
            pl.BlockSpec((WS, C, 512), lambda a: (strip(a), 0, 0)),
            pl.BlockSpec((1, C, 512), lambda a: (jnp.maximum(strip(a) * WS - 1, 0), 0, 0)),
            pl.BlockSpec((1, C, 512), lambda a: (jnp.minimum(strip(a) * WS + WS, H - 1), 0, 0)),
            full((9, C)),
            full((C, 3 * C)),
            full((C, C)),
        ],
        out_specs=pl.BlockSpec((WS, C, 512), lambda a: (jnp.maximum(a - 2, 0), 0, 0)),
        out_shape=jax.ShapeDtypeStruct((H, C, W), x.dtype),
        scratch_shapes=[
            pltpu.VMEM((9, 2, CW, 128), F32),
            pltpu.VMEM((128, 640), U32),
            pltpu.VMEM((CW, 256), U32),
            pltpu.VMEM((WS, 2, CW, 512), F32),
            pltpu.VMEM((WS, CW, 512), U32),
            pltpu.VMEM((WS, 2, 256, 128), U32),
            pltpu.VMEM((WS, 6, 512, 128), U32),
            pltpu.VMEM((WS, 2, 512, 128), F32),
            pltpu.SMEM((1,), jnp.int32),
        ],
        compiler_params=pltpu.CompilerParams(
            dimension_semantics=("arbitrary",),
            vmem_limit_bytes=100 * 1024 * 1024,
        ),
    )(xt, xt, xt, dw, w_qkv, w_o)
    return jnp.transpose(out.reshape(B, H, C, W), (0, 1, 3, 2))
```

```python
import functools

import jax
import jax.numpy as jnp
import jax.experimental.pallas as pl
import jax.experimental.pallas.tpu as pltpu
from jax import lax

WS = 7
NH = 4
C = 192
DH = C // NH
CW = C // 2
F32 = jnp.float32
BF16 = jnp.bfloat16
U32 = jnp.uint32
NT_DIMS = (((1,), (1,)), ((), ()))
NN_DIMS = (((1,), (0,)), ((), ()))
NEG = -1e30
LOG2E = 1.4426950408889634
UW = 8
SKEW = 1
LEAD = 2
PSPLIT = 1
FLAGS = None
QORDER = (0, 1, 2, 3, 4)
XLEAD = 2
PSPLIT = 1
FLAGS = None
OLEAD = 2
PSPLIT = 1
FLAGS = None
QORDER = (0, 1, 2, 3, 4)
OPRE = 0
EXP_LIMIT = 40.0
UC = 2
APPROX = True


def _dot(a, b, dims=NN_DIMS):
    return lax.dot_general(a, b, dims, preferred_element_type=F32)


def _iota(shape, dim):
    return lax.broadcasted_iota(jnp.int32, shape, dim)


def _f32(words):
    return pltpu.bitcast(words, F32)


def _lo(words):
    return _f32(words << 16)


def _hi(words):
    return _f32(words & U32(0xFFFF0000))


def _pack2(a, b):
    return pltpu.pack_elementwise([a, b], packed_dtype=BF16)


def _onehot(rows_map, cols_map):
    return jnp.where(rows_map == cols_map, 1.0, 0.0).astype(BF16)


def _prepare_weights(dw_ref, wqkv_ref, wo_ref, dwt_ref, wq_ref, wot_ref):
    r_i = _iota((CW, C), 0)
    c_i = _iota((CW, C), 1)
    for p in range(2):
        sel = _onehot(2 * r_i + p, c_i)
        for k in range(9):
            rep = jnp.broadcast_to(dw_ref[k:k + 1, :], (128, C))
            t = _dot(sel, rep, NT_DIMS)
            if k == 4:
                t = t + 1.0
            dwt_ref[k, p] = t
    rho = _iota((256, C), 0)
    rr = rho & 127
    chan = jnp.where(rr < CW, 2 * rr + (rho >> 7), -1)
    rsel = _onehot(chan, _iota((256, C), 1))
    w1 = _dot(rsel, wqkv_ref[...]).astype(BF16)
    n = _iota((3 * C, 640), 1)
    l = n & 127
    t = n >> 7
    col0 = jnp.where(l < 96, l, 384 + 64 + l - 96)
    col1 = jnp.where(l >= 32, 96 + l - 32, 384 + l)
    col2 = jnp.where(l < 96, 192 + l, -1)
    col3 = jnp.where(l >= 32, 288 + l - 32, -1)
    col4 = jnp.where(l < 32, 480 + l, jnp.where(l < 64, 384 + l, 448 + l))
    col = jnp.where(t == 0, col0, jnp.where(t == 1, col1, jnp.where(t == 2, col2,
                    jnp.where(t == 3, col3, col4))))
    csel = _onehot(_iota((3 * C, 640), 0), col)
    wq = _dot(w1, csel)
    wq_ref[...] = pltpu.bitcast(wq.astype(BF16), U32)
    lam = _iota((256, C), 0)
    ll = lam & 127
    fa = jnp.where(ll < 64, ll, jnp.where(ll < 96, -1, ll - 32))
    fb = jnp.where(ll < 32, 96 + ll, jnp.where(ll < 64, -1, 64 + ll))
    feat = jnp.where(lam < 128, fa, fb)
    fsel = _onehot(feat, _iota((256, C), 1))
    tmp = _dot(fsel, wo_ref[...]).astype(BF16)
    rp = _iota((C, C), 0)
    ochan = jnp.where(rp < CW, 2 * rp, 2 * (rp - CW) + 1)
    osel = _onehot(ochan, _iota((C, C), 1))
    wot_ref[...] = pltpu.bitcast(_dot(osel, tmp, NT_DIMS).astype(BF16), U32)


def _kernel(xm_ref, xt_ref, xb_ref, dw_ref, wqkv_ref, wo_ref, o_ref,
            dwt_ref, wq_ref, wot_ref, x0_ref, res_ref, hs_ref, qkv_ref, os_ref, flag_ref,
            *, n_strips, width):
    s = pl.program_id(0)
    WP = 512
    NTILE = WS * 4

    sub = _iota((8, 128), 0)
    lane = _iota((8, 128), 1)
    lo16, hi16 = U32(0x0000FFFF), U32(0xFFFF0000)
    zero = U32(0)

    def rows(m, n):
        return jnp.concatenate([m] * n, axis=0)

    def halves(hp0, hp1):
        return jnp.where(hp0, lo16, jnp.where(hp1, hi16, zero))

    key_ok = sub < WS
    kmask = [halves(lane < 48, (lane >= 48) & (lane < 96)),
             halves((lane >= 32) & (lane < 80), lane >= 80)]
    va1 = ((lane >= 48) & (lane < 64)) | (lane >= 96)
    vb1 = lane >= 80
    vmask = [halves(lane < 48, va1), halves((lane < 32) | ((lane >= 64) & (lane < 80)), vb1)]
    key_mask = jnp.where(key_ok, U32(0xFFFFFFFF), zero)
    one_lo, one_hi = U32(0x00003F80), U32(0x3F800000)

    def ones(d0):
        m = jnp.where((lane >= d0) & (lane < d0 + 16), one_lo,
                      jnp.where((lane >= d0 + 16) & (lane < d0 + 32), one_hi, zero))
        return m

    vones = [ones(64), ones(32)]
    den_idx = [jnp.where(va1, 80, 64), jnp.where(vb1, 48, 32)]
    even = (lane & 1) == 0
    s_valid = ((lane & 15) < 14) & (lane < 112)
    quarter = lane >> 5
    last_valid = lane < (width - 384)
    c_exp = (DH ** -0.5) * LOG2E

    def conv_steps(g):
        top_ok = s > 0
        bot_ok = s < n_strips - 1
        c0 = g * 16 if isinstance(g, int) else pl.multiple_of(g * 16, 16)
        r0 = g * 8 if isinstance(g, int) else pl.multiple_of(g * 8, 8)
        for p, unp in enumerate((_lo, _hi)):
            taps = [dwt_ref[k, p, pl.ds(r0, 8), :] for k in range(9)]
            xs = {}
            for r in range(-1, WS + 1):
                if r == -1:
                    raw = xt_ref[0, pl.ds(c0, 16), :]
                elif r == WS:
                    raw = xb_ref[0, pl.ds(c0, 16), :]
                else:
                    raw = xm_ref[r, pl.ds(c0, 16), :]
                w = pltpu.bitcast(raw, U32)
                w = jnp.concatenate([w[:, :384], jnp.where(last_valid, w[:, 384:], zero)], axis=1)
                if r == -1:
                    w = jnp.where(top_ok, w, zero)
                if r == WS:
                    w = jnp.where(bot_ok, w, zero)
                xs[r] = [unp(w[:, 128 * L:128 * L + 128]) for L in range(4)]
                if r >= 1:
                    i = r - 1
                    t = [jnp.concatenate(
                        [xs[i - 1][L] * taps[j] + xs[i][L] * taps[3 + j] + xs[i + 1][L] * taps[6 + j]
                         for L in range(4)], axis=1) for j in range(3)]
                    x0_ref[i, p, pl.ds(r0, 8), :] = (
                        pltpu.roll(t[0], 1, 1) + t[1] + pltpu.roll(t[2], WP - 1, 1))
                    del xs[i - 1]
                if p == 1 or not PSPLIT:
                    yield

    def conv_group(g):
        for _ in conv_steps(g):
            pass

    def tile_pos(it):
        if isinstance(it, int):
            return it // 4, (it % 4) * 128
        return it >> 2, pl.multiple_of((it & 3) * 128, 128)

    def ln_tile(it):
        i, l0 = tile_pos(it)
        xe = x0_ref[i, 0, :, pl.ds(l0, 128)]
        xo = x0_ref[i, 1, :, pl.ds(l0, 128)]
        res_ref[i, :, pl.ds(l0, 128)] = _pack2(xe, xo)
        mean = jnp.sum(xe + xo, axis=0, keepdims=True) * (1.0 / C)
        de = xe - mean
        do = xo - mean
        var = jnp.sum(de * de + do * do, axis=0, keepdims=True) * (1.0 / C)
        rstd = lax.rsqrt(var + 1e-5)
        return _pack2(de * rstd, do * rstd)

    def xpose_tile(it, words):
        i, l0 = tile_pos(it)
        words = jnp.concatenate([words, jnp.zeros((128 - CW, 128), U32)], axis=0)
        words = words.T
        t0 = l0 // 2 if isinstance(l0, int) else pl.multiple_of(l0 >> 1, 64)
        for p, unp in enumerate((_lo, _hi)):
            hs_ref[i, p, pl.ds(t0, 64), :] = pltpu.bitcast(unp(words).astype(BF16), U32)

    def qkv_tile(it):
        i, l0 = tile_pos(it)
        t0 = l0 // 2 if isinstance(l0, int) else pl.multiple_of(l0 >> 1, 64)
        he = pltpu.bitcast(hs_ref[i, 0, pl.ds(t0, 64), :], BF16)
        ho = pltpu.bitcast(hs_ref[i, 1, pl.ds(t0, 64), :], BF16)
        q16 = rows(quarter, 16)
        dst = lambda j: qkv_ref.at[i, j, pl.ds(l0, 128), :]
        for j in QORDER:
            we = pltpu.bitcast(wq_ref[0:64, 128 * j:128 * (j + 1)], BF16)
            wo = pltpu.bitcast(wq_ref[64:128, 128 * j:128 * (j + 1)], BF16)
            t = _dot(he, we) + _dot(ho, wo)
            if j == 4:
                w = _pack2(t, t)
                dst(5)[...] = (w & rows(vmask[1], 16)) | rows(vones[1], 16)
                pltpu.store(dst(4), w & rows(vmask[0], 16), mask=q16 == 1)
                pltpu.store(dst(4), rows(vones[0], 16), mask=q16 == 2)
            elif j < 2:
                dst(j)[...] = pltpu.bitcast(t * c_exp, U32)
                pltpu.store(dst(4), _pack2(t, t) & rows(vmask[0], 16), mask=q16 == (3 if j == 0 else 0))
            else:
                dst(j)[...] = _pack2(t, t) & rows(kmask[j - 2], 16)

    zpad = jnp.zeros((16, 128), BF16)

    def gather(j, off):
        return jnp.concatenate([qkv_ref[i, j, pl.ds(off, 8), :] for i in range(WS)], axis=0)

    def scores(off, exact_max):
        ps = []
        for pr in range(2):
            q = _f32(gather(pr, off))
            kbd = jnp.concatenate([pltpu.bitcast(gather(2 + pr, off), BF16), zpad], axis=0)
            sc = _dot(q, kbd, NT_DIMS)
            if exact_max:
                sc = jnp.where(rows(s_valid, WS), sc, NEG)
                ev = rows(even, WS)
                m0 = jnp.max(jnp.where(ev, sc, NEG), axis=1, keepdims=True)
                m1 = jnp.max(jnp.where(ev, NEG, sc), axis=1, keepdims=True)
                sc = sc - jnp.where(ev, m0, m1)
            ps.append(jnp.exp2(sc))
        return ps

    def attend(off, ps):
        for pr in range(2):
            vw = gather(4 + pr, off) & rows(key_mask, WS)
            vbd = jnp.concatenate([pltpu.bitcast(vw, BF16), zpad], axis=0)
            o = _dot(ps[pr], vbd)
            for i in range(WS):
                os_ref[i, pr, pl.ds(off, 8), :] = o[8 * i:8 * i + 8, :]

    n_win = width // WS

    def attention_fast():
        steps = (None for gg in range(CW // 8) for _ in conv_steps(gg))
        n_steps = (CW // 8) * (WS + 2)
        pend = [scores(WS * w, False) for w in range(SKEW)]
        g = 0
        for w in range(n_win):
            if w + SKEW < n_win:
                pend.append(scores(WS * (w + SKEW), False))
            attend(WS * w, pend.pop(0))
            while g * n_win < (w + 1) * n_steps:
                next(steps, None)
                g += 1
        for _ in steps:
            pass

    def attention_exact():
        def body(qi, ps):
            base = pl.multiple_of(qi * (8 * WS), 8)
            for u in range(8):
                nxt = scores(base + WS * (u + 1), True)
                attend(base + WS * u, ps)
                ps = nxt
            return ps
        n_it = (n_win - 1) // 8
        ps = lax.fori_loop(0, n_it, body, scores(0, True))
        for w in range(n_it * 8, n_win):
            nxt = scores(WS * (w + 1), True) if w + 1 < n_win else None
            attend(WS * w, ps)
            ps = nxt
        conv_only()

    def out_load(it):
        i, l0 = tile_pos(it)
        ob = []
        for pr in range(2):
            o = os_ref[i, pr, pl.ds(l0, 128), :]
            den = jnp.take_along_axis(o, rows(den_idx[pr], 16), axis=1, mode="promise_in_bounds")
            ob.append((o * pltpu.reciprocal(den, approx=APPROX, full_range=False)).astype(BF16))
        return ob, res_ref[i, :, pl.ds(l0, 128)]

    def out_tile(it, pre=None):
        i, l0 = tile_pos(it)
        (oa, ob), rw = out_load(it) if pre is None else pre
        wa = pltpu.bitcast(wot_ref[:, 0:128], BF16)
        wb = pltpu.bitcast(wot_ref[:, 128:256], BF16)
        y = _dot(wa, oa, NT_DIMS) + _dot(wb, ob, NT_DIMS)
        ye = y[0:CW] + _lo(rw)
        yo = y[CW:C] + _hi(rw)
        o_ref[i, :, pl.ds(l0, 128)] = pltpu.bitcast(_pack2(ye, yo), BF16)

    def conv_only():
        def body(g, c):
            conv_group(g)
            return c
        lax.fori_loop(0, CW // 8, body, 0)

    def out_only():
        def body(it, c):
            pre = [out_load(4 * it + u) for u in range(4)]
            for u in range(4):
                out_tile(4 * it + u, pre[u])
            return c
        lax.fori_loop(0, NTILE // 4, body, 0)

    def phase_b():
        words, pre = {}, {}
        for it in range(-LEAD, NTILE):
            t = it + OLEAD + OPRE
            if 0 <= t < NTILE:
                pre[t] = out_load(t)
            t = it + OLEAD
            if 0 <= t < NTILE:
                out_tile(t, pre.pop(t))
            t = it + LEAD
            if 0 <= t < NTILE:
                words[t] = ln_tile(t)
            t = it + XLEAD
            if 0 <= t < NTILE:
                xpose_tile(t, words.pop(t))
            if it >= 0:
                qkv_tile(it)

    @pl.when(s == 0)
    def _():
        _prepare_weights(dw_ref, wqkv_ref, wo_ref, dwt_ref, wq_ref, wot_ref)
        wq = pltpu.bitcast(wq_ref[...], BF16).astype(F32)
        sq = jnp.sum(wq * wq, axis=0, keepdims=True)
        l640 = _iota((1, 640), 1)
        t640, l128 = l640 >> 7, l640 & 127

        def norm2(tile, lo, hi):
            return jnp.sum(jnp.where((t640 == tile) & (l128 >= lo) & (l128 < hi), sq, 0.0))
        heads = [(0, 2, 0, 48), (0, 2, 48, 96), (1, 3, 32, 80), (1, 3, 80, 128)]
        bound2 = 0.0
        for tq, tk, lo, hi in heads:
            bound2 = jnp.maximum(bound2, norm2(tq, lo, hi) * norm2(tk, lo, hi))
        safe = bound2 * (1.1 * C * c_exp) ** 2 <= EXP_LIMIT ** 2
        flag_ref[0] = jnp.where(safe, 1, 0).astype(jnp.int32)
        os_ref[...] = jnp.ones(os_ref.shape, F32)
        res_ref[...] = jnp.zeros(res_ref.shape, U32)
        conv_only()

    @pl.when((s > 0) & (s <= n_strips))
    def _():
        phase_b()
        safe = flag_ref[0] == 1

        @pl.when(safe)
        def _():
            attention_fast()

        @pl.when(jnp.logical_not(safe))
        def _():
            attention_exact()

    @pl.when(s == n_strips + 1)
    def _():
        out_only()


@jax.jit
def pallas_standalone__window_attn_davit__vision_kernel(
    x: jax.Array,
    dw_pe: jax.Array,
    w_qkv: jax.Array,
    w_o: jax.Array,
):
    B, H, W, Cc = x.shape
    assert B == 1 and Cc == C and dw_pe.shape == (3, 3, C)
    assert H % WS == 0 and W % WS == 0 and 384 < W <= 512
    n_strips = H // WS
    xt = jnp.transpose(x, (0, 1, 3, 2)).reshape(H, C, W)
    dw = dw_pe.reshape(9, C)

    strip = lambda a: jnp.minimum(a, n_strips - 1)
    full = lambda shape: pl.BlockSpec(shape, lambda a: (0,) * len(shape))
    out = pl.pallas_call(
        functools.partial(_kernel, n_strips=n_strips, width=W),
        grid=(n_strips + 2,),
        in_specs=[
            pl.BlockSpec((WS, C, 512), lambda a: (strip(a), 0, 0)),
            pl.BlockSpec((1, C, 512), lambda a: (jnp.maximum(strip(a) * WS - 1, 0), 0, 0)),
            pl.BlockSpec((1, C, 512), lambda a: (jnp.minimum(strip(a) * WS + WS, H - 1), 0, 0)),
            full((9, C)),
            full((C, 3 * C)),
            full((C, C)),
        ],
        out_specs=pl.BlockSpec((WS, C, 512), lambda a: (jnp.maximum(a - 2, 0), 0, 0)),
        out_shape=jax.ShapeDtypeStruct((H, C, W), x.dtype),
        scratch_shapes=[
            pltpu.VMEM((9, 2, CW, 128), F32),
            pltpu.VMEM((128, 640), U32),
            pltpu.VMEM((CW, 256), U32),
            pltpu.VMEM((WS, 2, CW, 512), F32),
            pltpu.VMEM((WS, CW, 512), U32),
            pltpu.VMEM((WS, 2, 256, 128), U32),
            pltpu.VMEM((WS, 6, 512, 128), U32),
            pltpu.VMEM((WS, 2, 512, 128), F32),
            pltpu.SMEM((1,), jnp.int32),
        ],
        compiler_params=pltpu.CompilerParams(
            dimension_semantics=("arbitrary",),
            vmem_limit_bytes=100 * 1024 * 1024,
            flags=FLAGS,
        ),
    )(xt, xt, xt, dw, w_qkv, w_o)
    return jnp.transpose(out.reshape(B, H, C, W), (0, 1, 3, 2))
```

```python
import functools

import jax
import jax.numpy as jnp
import jax.experimental.pallas as pl
import jax.experimental.pallas.tpu as pltpu
from jax import lax

WS = 7
NH = 4
C = 192
DH = C // NH
CW = C // 2
F32 = jnp.float32
BF16 = jnp.bfloat16
U32 = jnp.uint32
NT_DIMS = (((1,), (1,)), ((), ()))
NN_DIMS = (((1,), (0,)), ((), ()))
NEG = -1e30
LOG2E = 1.4426950408889634
UW = 8
SKEW = 1
LEAD = 2
PSPLIT = 1
FLAGS = {'XLA_TPU_EVENLY_DISTRIBUTE_CRITICAL_NODES': True}
MOVE = 1
QORDER = (0, 1, 2, 3, 4)
XLEAD = 2
PSPLIT = 1
FLAGS = {'XLA_TPU_EVENLY_DISTRIBUTE_CRITICAL_NODES': True}
MOVE = 1
OLEAD = 2
PSPLIT = 1
FLAGS = {'XLA_TPU_EVENLY_DISTRIBUTE_CRITICAL_NODES': True}
MOVE = 1
QORDER = (0, 1, 2, 3, 4)
OPRE = 0
EXP_LIMIT = 40.0
UC = 2
APPROX = True


def _dot(a, b, dims=NN_DIMS):
    return lax.dot_general(a, b, dims, preferred_element_type=F32)


def _iota(shape, dim):
    return lax.broadcasted_iota(jnp.int32, shape, dim)


def _f32(words):
    return pltpu.bitcast(words, F32)


def _lo(words):
    return _f32(words << 16)


def _hi(words):
    return _f32(words & U32(0xFFFF0000))


def _pack2(a, b):
    return pltpu.pack_elementwise([a, b], packed_dtype=BF16)


def _onehot(rows_map, cols_map):
    return jnp.where(rows_map == cols_map, 1.0, 0.0).astype(BF16)


def _prepare_weights(dw_ref, wqkv_ref, wo_ref, dwt_ref, wq_ref, wot_ref):
    r_i = _iota((CW, C), 0)
    c_i = _iota((CW, C), 1)
    for p in range(2):
        sel = _onehot(2 * r_i + p, c_i)
        for k in range(9):
            rep = jnp.broadcast_to(dw_ref[k:k + 1, :], (128, C))
            t = _dot(sel, rep, NT_DIMS)
            if k == 4:
                t = t + 1.0
            dwt_ref[k, p] = t
    rho = _iota((256, C), 0)
    rr = rho & 127
    chan = jnp.where(rr < CW, 2 * rr + (rho >> 7), -1)
    rsel = _onehot(chan, _iota((256, C), 1))
    w1 = _dot(rsel, wqkv_ref[...]).astype(BF16)
    n = _iota((3 * C, 640), 1)
    l = n & 127
    t = n >> 7
    col0 = jnp.where(l < 96, l, 384 + 64 + l - 96)
    col1 = jnp.where(l >= 32, 96 + l - 32, 384 + l)
    col2 = jnp.where(l < 96, 192 + l, -1)
    col3 = jnp.where(l >= 32, 288 + l - 32, -1)
    col4 = jnp.where(l < 32, 480 + l, jnp.where(l < 64, 384 + l, 448 + l))
    col = jnp.where(t == 0, col0, jnp.where(t == 1, col1, jnp.where(t == 2, col2,
                    jnp.where(t == 3, col3, col4))))
    csel = _onehot(_iota((3 * C, 640), 0), col)
    wq = _dot(w1, csel)
    wq_ref[...] = pltpu.bitcast(wq.astype(BF16), U32)
    lam = _iota((256, C), 0)
    ll = lam & 127
    fa = jnp.where(ll < 64, ll, jnp.where(ll < 96, -1, ll - 32))
    fb = jnp.where(ll < 32, 96 + ll, jnp.where(ll < 64, -1, 64 + ll))
    feat = jnp.where(lam < 128, fa, fb)
    fsel = _onehot(feat, _iota((256, C), 1))
    tmp = _dot(fsel, wo_ref[...]).astype(BF16)
    rp = _iota((C, C), 0)
    ochan = jnp.where(rp < CW, 2 * rp, 2 * (rp - CW) + 1)
    osel = _onehot(ochan, _iota((C, C), 1))
    wot_ref[...] = pltpu.bitcast(_dot(osel, tmp, NT_DIMS).astype(BF16), U32)


def _kernel(xm_ref, xt_ref, xb_ref, dw_ref, wqkv_ref, wo_ref, o_ref,
            dwt_ref, wq_ref, wot_ref, x0_ref, res_ref, hs_ref, qkv_ref, os_ref, flag_ref,
            *, n_strips, width):
    s = pl.program_id(0)
    WP = 512
    NTILE = WS * 4
    rslot = (s & 1) if MOVE else 0

    sub = _iota((8, 128), 0)
    lane = _iota((8, 128), 1)
    lo16, hi16 = U32(0x0000FFFF), U32(0xFFFF0000)
    zero = U32(0)

    def rows(m, n):
        return jnp.concatenate([m] * n, axis=0)

    def halves(hp0, hp1):
        return jnp.where(hp0, lo16, jnp.where(hp1, hi16, zero))

    key_ok = sub < WS
    kmask = [halves(lane < 48, (lane >= 48) & (lane < 96)),
             halves((lane >= 32) & (lane < 80), lane >= 80)]
    va1 = ((lane >= 48) & (lane < 64)) | (lane >= 96)
    vb1 = lane >= 80
    vmask = [halves(lane < 48, va1), halves((lane < 32) | ((lane >= 64) & (lane < 80)), vb1)]
    key_mask = jnp.where(key_ok, U32(0xFFFFFFFF), zero)
    one_lo, one_hi = U32(0x00003F80), U32(0x3F800000)

    def ones(d0):
        m = jnp.where((lane >= d0) & (lane < d0 + 16), one_lo,
                      jnp.where((lane >= d0 + 16) & (lane < d0 + 32), one_hi, zero))
        return m

    vones = [ones(64), ones(32)]
    den_idx = [jnp.where(va1, 80, 64), jnp.where(vb1, 48, 32)]
    even = (lane & 1) == 0
    s_valid = ((lane & 15) < 14) & (lane < 112)
    quarter = lane >> 5
    last_valid = lane < (width - 384)
    c_exp = (DH ** -0.5) * LOG2E

    def conv_steps(g):
        top_ok = s > 0
        bot_ok = s < n_strips - 1
        c0 = g * 16 if isinstance(g, int) else pl.multiple_of(g * 16, 16)
        r0 = g * 8 if isinstance(g, int) else pl.multiple_of(g * 8, 8)
        for p, unp in enumerate((_lo, _hi)):
            taps = [dwt_ref[k, p, pl.ds(r0, 8), :] for k in range(9)]
            xs = {}
            for r in range(-1, WS + 1):
                if r == -1:
                    raw = xt_ref[0, pl.ds(c0, 16), :]
                elif r == WS:
                    raw = xb_ref[0, pl.ds(c0, 16), :]
                else:
                    raw = xm_ref[r, pl.ds(c0, 16), :]
                w = pltpu.bitcast(raw, U32)
                w = jnp.concatenate([w[:, :384], jnp.where(last_valid, w[:, 384:], zero)], axis=1)
                if r == -1:
                    w = jnp.where(top_ok, w, zero)
                if r == WS:
                    w = jnp.where(bot_ok, w, zero)
                xs[r] = [unp(w[:, 128 * L:128 * L + 128]) for L in range(4)]
                if r >= 1:
                    i = r - 1
                    t = [jnp.concatenate(
                        [xs[i - 1][L] * taps[j] + xs[i][L] * taps[3 + j] + xs[i + 1][L] * taps[6 + j]
                         for L in range(4)], axis=1) for j in range(3)]
                    x0_ref[i, p, pl.ds(r0, 8), :] = (
                        pltpu.roll(t[0], 1, 1) + t[1] + pltpu.roll(t[2], WP - 1, 1))
                    del xs[i - 1]
                if p == 1 or not PSPLIT:
                    yield

    def conv_group(g):
        for _ in conv_steps(g):
            pass

    def tile_pos(it):
        if isinstance(it, int):
            return it // 4, (it % 4) * 128
        return it >> 2, pl.multiple_of((it & 3) * 128, 128)

    def ln_tile(it):
        i, l0 = tile_pos(it)
        xe = x0_ref[i, 0, :, pl.ds(l0, 128)]
        xo = x0_ref[i, 1, :, pl.ds(l0, 128)]
        res_ref[rslot, i, :, pl.ds(l0, 128)] = _pack2(xe, xo)
        mean = jnp.sum(xe + xo, axis=0, keepdims=True) * (1.0 / C)
        de = xe - mean
        do = xo - mean
        var = jnp.sum(de * de + do * do, axis=0, keepdims=True) * (1.0 / C)
        rstd = lax.rsqrt(var + 1e-5)
        return _pack2(de * rstd, do * rstd)

    def xpose_tile(it, words):
        i, l0 = tile_pos(it)
        words = jnp.concatenate([words, jnp.zeros((128 - CW, 128), U32)], axis=0)
        words = words.T
        t0 = l0 // 2 if isinstance(l0, int) else pl.multiple_of(l0 >> 1, 64)
        for p, unp in enumerate((_lo, _hi)):
            hs_ref[i, p, pl.ds(t0, 64), :] = pltpu.bitcast(unp(words).astype(BF16), U32)

    def qkv_tile(it):
        i, l0 = tile_pos(it)
        t0 = l0 // 2 if isinstance(l0, int) else pl.multiple_of(l0 >> 1, 64)
        he = pltpu.bitcast(hs_ref[i, 0, pl.ds(t0, 64), :], BF16)
        ho = pltpu.bitcast(hs_ref[i, 1, pl.ds(t0, 64), :], BF16)
        q16 = rows(quarter, 16)
        dst = lambda j: qkv_ref.at[i, j, pl.ds(l0, 128), :]
        for j in QORDER:
            we = pltpu.bitcast(wq_ref[0:64, 128 * j:128 * (j + 1)], BF16)
            wo = pltpu.bitcast(wq_ref[64:128, 128 * j:128 * (j + 1)], BF16)
            t = _dot(he, we) + _dot(ho, wo)
            if j == 4:
                w = _pack2(t, t)
                dst(5)[...] = (w & rows(vmask[1], 16)) | rows(vones[1], 16)
                pltpu.store(dst(4), w & rows(vmask[0], 16), mask=q16 == 1)
                pltpu.store(dst(4), rows(vones[0], 16), mask=q16 == 2)
            elif j < 2:
                dst(j)[...] = pltpu.bitcast(t * c_exp, U32)
                pltpu.store(dst(4), _pack2(t, t) & rows(vmask[0], 16), mask=q16 == (3 if j == 0 else 0))
            else:
                dst(j)[...] = _pack2(t, t) & rows(kmask[j - 2], 16)

    zpad = jnp.zeros((16, 128), BF16)

    def gather(j, off):
        return jnp.concatenate([qkv_ref[i, j, pl.ds(off, 8), :] for i in range(WS)], axis=0)

    def scores(off, exact_max):
        ps = []
        for pr in range(2):
            q = _f32(gather(pr, off))
            kbd = jnp.concatenate([pltpu.bitcast(gather(2 + pr, off), BF16), zpad], axis=0)
            sc = _dot(q, kbd, NT_DIMS)
            if exact_max:
                sc = jnp.where(rows(s_valid, WS), sc, NEG)
                ev = rows(even, WS)
                m0 = jnp.max(jnp.where(ev, sc, NEG), axis=1, keepdims=True)
                m1 = jnp.max(jnp.where(ev, NEG, sc), axis=1, keepdims=True)
                sc = sc - jnp.where(ev, m0, m1)
            ps.append(jnp.exp2(sc))
        return ps

    def attend(off, ps):
        for pr in range(2):
            vw = gather(4 + pr, off) & rows(key_mask, WS)
            vbd = jnp.concatenate([pltpu.bitcast(vw, BF16), zpad], axis=0)
            o = _dot(ps[pr], vbd)
            for i in range(WS):
                os_ref[i, pr, pl.ds(off, 8), :] = o[8 * i:8 * i + 8, :]

    n_win = width // WS

    def attention_fast():
        if MOVE:
            steps = (xpose_tile(t, ln_tile(t)) for t in range(NTILE))
            n_steps = NTILE
        else:
            steps = (None for gg in range(CW // 8) for _ in conv_steps(gg))
            n_steps = (CW // 8) * (WS + 2)
        pend = [scores(WS * w, False) for w in range(SKEW)]
        g = 0
        for w in range(n_win):
            if w + SKEW < n_win:
                pend.append(scores(WS * (w + SKEW), False))
            attend(WS * w, pend.pop(0))
            while g * n_win < (w + 1) * n_steps:
                next(steps, None)
                g += 1
        for _ in steps:
            pass

    def attention_exact():
        def body(qi, ps):
            base = pl.multiple_of(qi * (8 * WS), 8)
            for u in range(8):
                nxt = scores(base + WS * (u + 1), True)
                attend(base + WS * u, ps)
                ps = nxt
            return ps
        n_it = (n_win - 1) // 8
        ps = lax.fori_loop(0, n_it, body, scores(0, True))
        for w in range(n_it * 8, n_win):
            nxt = scores(WS * (w + 1), True) if w + 1 < n_win else None
            attend(WS * w, ps)
            ps = nxt
        ln_only() if MOVE else conv_only()

    def out_load(it):
        i, l0 = tile_pos(it)
        ob = []
        for pr in range(2):
            o = os_ref[i, pr, pl.ds(l0, 128), :]
            den = jnp.take_along_axis(o, rows(den_idx[pr], 16), axis=1, mode="promise_in_bounds")
            ob.append((o * pltpu.reciprocal(den, approx=APPROX, full_range=False)).astype(BF16))
        return ob, res_ref[rslot, i, :, pl.ds(l0, 128)]

    def out_tile(it, pre=None):
        i, l0 = tile_pos(it)
        (oa, ob), rw = out_load(it) if pre is None else pre
        wa = pltpu.bitcast(wot_ref[:, 0:128], BF16)
        wb = pltpu.bitcast(wot_ref[:, 128:256], BF16)
        y = _dot(wa, oa, NT_DIMS) + _dot(wb, ob, NT_DIMS)
        ye = y[0:CW] + _lo(rw)
        yo = y[CW:C] + _hi(rw)
        o_ref[i, :, pl.ds(l0, 128)] = pltpu.bitcast(_pack2(ye, yo), BF16)

    def conv_only():
        def body(g, c):
            conv_group(g)
            return c
        lax.fori_loop(0, CW // 8, body, 0)

    def ln_only():
        def body(it, c):
            words = [ln_tile(4 * it + u) for u in range(4)]
            for u in range(4):
                xpose_tile(4 * it + u, words[u])
            return c
        lax.fori_loop(0, NTILE // 4, body, 0)

    def out_only():
        def body(it, c):
            pre = [out_load(4 * it + u) for u in range(4)]
            for u in range(4):
                out_tile(4 * it + u, pre[u])
            return c
        lax.fori_loop(0, NTILE // 4, body, 0)

    def phase_b_move():
        steps = (None for gg in range(CW // 8) for _ in conv_steps(gg))
        n_steps = (CW // 8) * (WS + 2)
        g = 0
        for it in range(NTILE):
            out_tile(it)
            qkv_tile(it)
            while g * NTILE < (it + 1) * n_steps:
                next(steps, None)
                g += 1
        for _ in steps:
            pass

    def phase_b():
        if MOVE:
            return phase_b_move()
        words, pre = {}, {}
        for it in range(-LEAD, NTILE):
            t = it + OLEAD + OPRE
            if 0 <= t < NTILE:
                pre[t] = out_load(t)
            t = it + OLEAD
            if 0 <= t < NTILE:
                out_tile(t, pre.pop(t))
            t = it + LEAD
            if 0 <= t < NTILE:
                words[t] = ln_tile(t)
            t = it + XLEAD
            if 0 <= t < NTILE:
                xpose_tile(t, words.pop(t))
            if it >= 0:
                qkv_tile(it)

    @pl.when(s == 0)
    def _():
        _prepare_weights(dw_ref, wqkv_ref, wo_ref, dwt_ref, wq_ref, wot_ref)
        wq = pltpu.bitcast(wq_ref[...], BF16).astype(F32)
        sq = jnp.sum(wq * wq, axis=0, keepdims=True)
        l640 = _iota((1, 640), 1)
        t640, l128 = l640 >> 7, l640 & 127

        def norm2(tile, lo, hi):
            return jnp.sum(jnp.where((t640 == tile) & (l128 >= lo) & (l128 < hi), sq, 0.0))
        heads = [(0, 2, 0, 48), (0, 2, 48, 96), (1, 3, 32, 80), (1, 3, 80, 128)]
        bound2 = 0.0
        for tq, tk, lo, hi in heads:
            bound2 = jnp.maximum(bound2, norm2(tq, lo, hi) * norm2(tk, lo, hi))
        safe = bound2 * (1.1 * C * c_exp) ** 2 <= EXP_LIMIT ** 2
        flag_ref[0] = jnp.where(safe, 1, 0).astype(jnp.int32)
        os_ref[...] = jnp.ones(os_ref.shape, F32)
        res_ref[...] = jnp.zeros(res_ref.shape, U32)
        conv_only()
        if MOVE:
            ln_only()

    @pl.when((s > 0) & (s <= n_strips))
    def _():
        phase_b()
        safe = flag_ref[0] == 1

        @pl.when(safe)
        def _():
            attention_fast()

        @pl.when(jnp.logical_not(safe))
        def _():
            attention_exact()

    @pl.when(s == n_strips + 1)
    def _():
        out_only()


@jax.jit
def pallas_standalone__window_attn_davit__vision_kernel(
    x: jax.Array,
    dw_pe: jax.Array,
    w_qkv: jax.Array,
    w_o: jax.Array,
):
    B, H, W, Cc = x.shape
    assert B == 1 and Cc == C and dw_pe.shape == (3, 3, C)
    assert H % WS == 0 and W % WS == 0 and 384 < W <= 512
    n_strips = H // WS
    xt = jnp.transpose(x, (0, 1, 3, 2)).reshape(H, C, W)
    dw = dw_pe.reshape(9, C)

    strip = lambda a: jnp.minimum(a, n_strips - 1)
    full = lambda shape: pl.BlockSpec(shape, lambda a: (0,) * len(shape))
    out = pl.pallas_call(
        functools.partial(_kernel, n_strips=n_strips, width=W),
        grid=(n_strips + 2,),
        in_specs=[
            pl.BlockSpec((WS, C, 512), lambda a: (strip(a), 0, 0)),
            pl.BlockSpec((1, C, 512), lambda a: (jnp.maximum(strip(a) * WS - 1, 0), 0, 0)),
            pl.BlockSpec((1, C, 512), lambda a: (jnp.minimum(strip(a) * WS + WS, H - 1), 0, 0)),
            full((9, C)),
            full((C, 3 * C)),
            full((C, C)),
        ],
        out_specs=pl.BlockSpec((WS, C, 512), lambda a: (jnp.maximum(a - 2, 0), 0, 0)),
        out_shape=jax.ShapeDtypeStruct((H, C, W), x.dtype),
        scratch_shapes=[
            pltpu.VMEM((9, 2, CW, 128), F32),
            pltpu.VMEM((128, 640), U32),
            pltpu.VMEM((CW, 256), U32),
            pltpu.VMEM((WS, 2, CW, 512), F32),
            pltpu.VMEM((1 + MOVE, WS, CW, 512), U32),
            pltpu.VMEM((WS, 2, 256, 128), U32),
            pltpu.VMEM((WS, 6, 512, 128), U32),
            pltpu.VMEM((WS, 2, 512, 128), F32),
            pltpu.SMEM((1,), jnp.int32),
        ],
        compiler_params=pltpu.CompilerParams(
            dimension_semantics=("arbitrary",),
            vmem_limit_bytes=100 * 1024 * 1024,
            flags=FLAGS,
        ),
    )(xt, xt, xt, dw, w_qkv, w_o)
    return jnp.transpose(out.reshape(B, H, C, W), (0, 1, 3, 2))
```

```python
import functools

import jax
import jax.numpy as jnp
import jax.experimental.pallas as pl
import jax.experimental.pallas.tpu as pltpu
from jax import lax

WS = 7
NH = 4
C = 192
DH = C // NH
CW = C // 2
F32 = jnp.float32
BF16 = jnp.bfloat16
U32 = jnp.uint32
NT_DIMS = (((1,), (1,)), ((), ()))
NN_DIMS = (((1,), (0,)), ((), ()))
NEG = -1e30
LOG2E = 1.4426950408889634
EXP_LIMIT = 40.0
QORDER = (4, 0, 1, 2, 3)
SKEW = 2
STATIC_OUT = 1
STATIC_PRO = 1
FLAGS = {"XLA_TPU_EVENLY_DISTRIBUTE_CRITICAL_NODES": True}


def _dot(a, b, dims=NN_DIMS):
    return lax.dot_general(a, b, dims, preferred_element_type=F32)


def _iota(shape, dim):
    return lax.broadcasted_iota(jnp.int32, shape, dim)


def _f32(words):
    return pltpu.bitcast(words, F32)


def _lo(words):
    return _f32(words << 16)


def _hi(words):
    return _f32(words & U32(0xFFFF0000))


def _pack2(a, b):
    return pltpu.pack_elementwise([a, b], packed_dtype=BF16)


def _onehot(rows_map, cols_map):
    return jnp.where(rows_map == cols_map, 1.0, 0.0).astype(BF16)


def _prepare_weights(dw_ref, wqkv_ref, wo_ref, dwt_ref, wq_ref, wot_ref):
    r_i = _iota((CW, C), 0)
    c_i = _iota((CW, C), 1)
    for p in range(2):
        sel = _onehot(2 * r_i + p, c_i)
        for k in range(9):
            rep = jnp.broadcast_to(dw_ref[k:k + 1, :], (128, C))
            t = _dot(sel, rep, NT_DIMS)
            if k == 4:
                t = t + 1.0
            dwt_ref[k, p] = t
    rho = _iota((256, C), 0)
    rr = rho & 127
    chan = jnp.where(rr < CW, 2 * rr + (rho >> 7), -1)
    rsel = _onehot(chan, _iota((256, C), 1))
    w1 = _dot(rsel, wqkv_ref[...]).astype(BF16)
    n = _iota((3 * C, 640), 1)
    l = n & 127
    t = n >> 7
    col0 = jnp.where(l < 96, l, 384 + 64 + l - 96)
    col1 = jnp.where(l >= 32, 96 + l - 32, 384 + l)
    col2 = jnp.where(l < 96, 192 + l, -1)
    col3 = jnp.where(l >= 32, 288 + l - 32, -1)
    col4 = jnp.where(l < 32, 480 + l, jnp.where(l < 64, 384 + l, 448 + l))
    col = jnp.where(t == 0, col0, jnp.where(t == 1, col1, jnp.where(t == 2, col2,
                    jnp.where(t == 3, col3, col4))))
    csel = _onehot(_iota((3 * C, 640), 0), col)
    wq = _dot(w1, csel)
    wq_ref[...] = pltpu.bitcast(wq.astype(BF16), U32)
    lam = _iota((256, C), 0)
    ll = lam & 127
    fa = jnp.where(ll < 64, ll, jnp.where(ll < 96, -1, ll - 32))
    fb = jnp.where(ll < 32, 96 + ll, jnp.where(ll < 64, -1, 64 + ll))
    feat = jnp.where(lam < 128, fa, fb)
    fsel = _onehot(feat, _iota((256, C), 1))
    tmp = _dot(fsel, wo_ref[...]).astype(BF16)
    rp = _iota((C, C), 0)
    ochan = jnp.where(rp < CW, 2 * rp, 2 * (rp - CW) + 1)
    osel = _onehot(ochan, _iota((C, C), 1))
    wot_ref[...] = pltpu.bitcast(_dot(osel, tmp, NT_DIMS).astype(BF16), U32)


def _kernel(xm_ref, xt_ref, xb_ref, dw_ref, wqkv_ref, wo_ref, o_ref,
            dwt_ref, wq_ref, wot_ref, x0_ref, res_ref, hs_ref, qkv_ref, os_ref, flag_ref,
            *, n_strips, width):
    s = pl.program_id(0)
    WP = 512
    NTILE = WS * 4
    rslot = s & 1

    sub = _iota((8, 128), 0)
    lane = _iota((8, 128), 1)
    lo16, hi16 = U32(0x0000FFFF), U32(0xFFFF0000)
    zero = U32(0)

    def rows(m, n):
        return jnp.concatenate([m] * n, axis=0)

    def halves(hp0, hp1):
        return jnp.where(hp0, lo16, jnp.where(hp1, hi16, zero))

    key_ok = sub < WS
    kmask = [halves(lane < 48, (lane >= 48) & (lane < 96)),
             halves((lane >= 32) & (lane < 80), lane >= 80)]
    va1 = ((lane >= 48) & (lane < 64)) | (lane >= 96)
    vb1 = lane >= 80
    vmask = [halves(lane < 48, va1), halves((lane < 32) | ((lane >= 64) & (lane < 80)), vb1)]
    key_mask = jnp.where(key_ok, U32(0xFFFFFFFF), zero)
    one_lo, one_hi = U32(0x00003F80), U32(0x3F800000)

    def ones(d0):
        m = jnp.where((lane >= d0) & (lane < d0 + 16), one_lo,
                      jnp.where((lane >= d0 + 16) & (lane < d0 + 32), one_hi, zero))
        return m

    vones = [ones(64), ones(32)]
    den_idx = [jnp.where(va1, 80, 64), jnp.where(vb1, 48, 32)]
    even = (lane & 1) == 0
    s_valid = ((lane & 15) < 14) & (lane < 112)
    quarter = lane >> 5
    last_valid = lane < (width - 384)
    c_exp = (DH ** -0.5) * LOG2E

    def conv_steps(g):
        top_ok = s > 0
        bot_ok = s < n_strips - 1
        c0 = g * 16 if isinstance(g, int) else pl.multiple_of(g * 16, 16)
        r0 = g * 8 if isinstance(g, int) else pl.multiple_of(g * 8, 8)
        for p, unp in enumerate((_lo, _hi)):
            taps = [dwt_ref[k, p, pl.ds(r0, 8), :] for k in range(9)]
            xs = {}
            for r in range(-1, WS + 1):
                if r == -1:
                    raw = xt_ref[0, pl.ds(c0, 16), :]
                elif r == WS:
                    raw = xb_ref[0, pl.ds(c0, 16), :]
                else:
                    raw = xm_ref[r, pl.ds(c0, 16), :]
                w = pltpu.bitcast(raw, U32)
                w = jnp.concatenate([w[:, :384], jnp.where(last_valid, w[:, 384:], zero)], axis=1)
                if r == -1:
                    w = jnp.where(top_ok, w, zero)
                if r == WS:
                    w = jnp.where(bot_ok, w, zero)
                xs[r] = [unp(w[:, 128 * L:128 * L + 128]) for L in range(4)]
                if r >= 1:
                    i = r - 1
                    t = [jnp.concatenate(
                        [xs[i - 1][L] * taps[j] + xs[i][L] * taps[3 + j] + xs[i + 1][L] * taps[6 + j]
                         for L in range(4)], axis=1) for j in range(3)]
                    x0_ref[i, p, pl.ds(r0, 8), :] = (
                        pltpu.roll(t[0], 1, 1) + t[1] + pltpu.roll(t[2], WP - 1, 1))
                    del xs[i - 1]
                if p == 1:
                    yield

    def conv_group(g):
        for _ in conv_steps(g):
            pass

    def tile_pos(it):
        if isinstance(it, int):
            return it // 4, (it % 4) * 128
        return it >> 2, pl.multiple_of((it & 3) * 128, 128)

    def ln_tile(it):
        i, l0 = tile_pos(it)
        xe = x0_ref[i, 0, :, pl.ds(l0, 128)]
        xo = x0_ref[i, 1, :, pl.ds(l0, 128)]
        res_ref[rslot, i, :, pl.ds(l0, 128)] = _pack2(xe, xo)
        mean = jnp.sum(xe + xo, axis=0, keepdims=True) * (1.0 / C)
        de = xe - mean
        do = xo - mean
        var = jnp.sum(de * de + do * do, axis=0, keepdims=True) * (1.0 / C)
        rstd = lax.rsqrt(var + 1e-5)
        return _pack2(de * rstd, do * rstd)

    def xpose_tile(it, words):
        i, l0 = tile_pos(it)
        words = jnp.concatenate([words, jnp.zeros((128 - CW, 128), U32)], axis=0)
        words = words.T
        t0 = l0 // 2 if isinstance(l0, int) else pl.multiple_of(l0 >> 1, 64)
        for p, unp in enumerate((_lo, _hi)):
            hs_ref[i, p, pl.ds(t0, 64), :] = pltpu.bitcast(unp(words).astype(BF16), U32)

    def qkv_tile(it):
        i, l0 = tile_pos(it)
        t0 = l0 // 2 if isinstance(l0, int) else pl.multiple_of(l0 >> 1, 64)
        he = pltpu.bitcast(hs_ref[i, 0, pl.ds(t0, 64), :], BF16)
        ho = pltpu.bitcast(hs_ref[i, 1, pl.ds(t0, 64), :], BF16)
        q16 = rows(quarter, 16)
        dst = lambda j: qkv_ref.at[i, j, pl.ds(l0, 128), :]
        for j in QORDER:
            we = pltpu.bitcast(wq_ref[0:64, 128 * j:128 * (j + 1)], BF16)
            wo = pltpu.bitcast(wq_ref[64:128, 128 * j:128 * (j + 1)], BF16)
            t = _dot(he, we) + _dot(ho, wo)
            if j == 4:
                w = _pack2(t, t)
                dst(5)[...] = (w & rows(vmask[1], 16)) | rows(vones[1], 16)
                pltpu.store(dst(4), w & rows(vmask[0], 16), mask=q16 == 1)
                pltpu.store(dst(4), rows(vones[0], 16), mask=q16 == 2)
            elif j < 2:
                dst(j)[...] = pltpu.bitcast(t * c_exp, U32)
                pltpu.store(dst(4), _pack2(t, t) & rows(vmask[0], 16), mask=q16 == (3 if j == 0 else 0))
            else:
                dst(j)[...] = _pack2(t, t) & rows(kmask[j - 2], 16)

    zpad = jnp.zeros((16, 128), BF16)

    def gather(j, off):
        return jnp.concatenate([qkv_ref[i, j, pl.ds(off, 8), :] for i in range(WS)], axis=0)

    def scores(off, exact_max):
        ps = []
        for pr in range(2):
            q = _f32(gather(pr, off))
            kbd = jnp.concatenate([pltpu.bitcast(gather(2 + pr, off), BF16), zpad], axis=0)
            sc = _dot(q, kbd, NT_DIMS)
            if exact_max:
                sc = jnp.where(rows(s_valid, WS), sc, NEG)
                ev = rows(even, WS)
                m0 = jnp.max(jnp.where(ev, sc, NEG), axis=1, keepdims=True)
                m1 = jnp.max(jnp.where(ev, NEG, sc), axis=1, keepdims=True)
                sc = sc - jnp.where(ev, m0, m1)
            ps.append(jnp.exp2(sc))
        return ps

    def attend(off, ps):
        for pr in range(2):
            vw = gather(4 + pr, off) & rows(key_mask, WS)
            vbd = jnp.concatenate([pltpu.bitcast(vw, BF16), zpad], axis=0)
            o = _dot(ps[pr], vbd)
            for i in range(WS):
                os_ref[i, pr, pl.ds(off, 8), :] = o[8 * i:8 * i + 8, :]

    n_win = width // WS

    def attention_fast():
        steps = (xpose_tile(t, ln_tile(t)) for t in range(NTILE))
        n_steps = NTILE
        pend = [scores(WS * w, False) for w in range(SKEW)]
        g = 0
        for w in range(n_win):
            if w + SKEW < n_win:
                pend.append(scores(WS * (w + SKEW), False))
            attend(WS * w, pend.pop(0))
            while g * n_win < (w + 1) * n_steps:
                next(steps, None)
                g += 1
        for _ in steps:
            pass

    def attention_exact():
        def body(qi, ps):
            base = pl.multiple_of(qi * (8 * WS), 8)
            for u in range(8):
                nxt = scores(base + WS * (u + 1), True)
                attend(base + WS * u, ps)
                ps = nxt
            return ps
        n_it = (n_win - 1) // 8
        ps = lax.fori_loop(0, n_it, body, scores(0, True))
        for w in range(n_it * 8, n_win):
            nxt = scores(WS * (w + 1), True) if w + 1 < n_win else None
            attend(WS * w, ps)
            ps = nxt
        ln_only()

    def out_load(it):
        i, l0 = tile_pos(it)
        ob = []
        for pr in range(2):
            o = os_ref[i, pr, pl.ds(l0, 128), :]
            den = jnp.take_along_axis(o, rows(den_idx[pr], 16), axis=1, mode="promise_in_bounds")
            ob.append((o * pltpu.reciprocal(den, approx=True, full_range=False)).astype(BF16))
        return ob, res_ref[rslot, i, :, pl.ds(l0, 128)]

    def out_tile(it, pre=None):
        i, l0 = tile_pos(it)
        (oa, ob), rw = out_load(it) if pre is None else pre
        wa = pltpu.bitcast(wot_ref[:, 0:128], BF16)
        wb = pltpu.bitcast(wot_ref[:, 128:256], BF16)
        y = _dot(wa, oa, NT_DIMS) + _dot(wb, ob, NT_DIMS)
        ye = y[0:CW] + _lo(rw)
        yo = y[CW:C] + _hi(rw)
        o_ref[i, :, pl.ds(l0, 128)] = pltpu.bitcast(_pack2(ye, yo), BF16)

    def conv_only():
        def body(g, c):
            conv_group(g)
            return c
        lax.fori_loop(0, CW // 8, body, 0)

    def ln_only():
        def body(it, c):
            words = [ln_tile(4 * it + u) for u in range(4)]
            for u in range(4):
                xpose_tile(4 * it + u, words[u])
            return c
        lax.fori_loop(0, NTILE // 4, body, 0)

    def out_only():
        if STATIC_OUT:
            for it in range(NTILE):
                out_tile(it)
            return

        def body(it, c):
            pre = [out_load(4 * it + u) for u in range(4)]
            for u in range(4):
                out_tile(4 * it + u, pre[u])
            return c
        lax.fori_loop(0, NTILE // 4, body, 0)

    def phase_b():
        steps = (None for gg in range(CW // 8) for _ in conv_steps(gg))
        n_steps = (CW // 8) * (WS + 2)
        g = 0
        for it in range(NTILE):
            out_tile(it)
            qkv_tile(it)
            while g * NTILE < (it + 1) * n_steps:
                next(steps, None)
                g += 1
        for _ in steps:
            pass

    @pl.when(s == 0)
    def _():
        _prepare_weights(dw_ref, wqkv_ref, wo_ref, dwt_ref, wq_ref, wot_ref)
        wq = pltpu.bitcast(wq_ref[...], BF16).astype(F32)
        sq = jnp.sum(wq * wq, axis=0, keepdims=True)
        l640 = _iota((1, 640), 1)
        t640, l128 = l640 >> 7, l640 & 127

        def norm2(tile, lo, hi):
            return jnp.sum(jnp.where((t640 == tile) & (l128 >= lo) & (l128 < hi), sq, 0.0))
        heads = [(0, 2, 0, 48), (0, 2, 48, 96), (1, 3, 32, 80), (1, 3, 80, 128)]
        bound2 = 0.0
        for tq, tk, lo, hi in heads:
            bound2 = jnp.maximum(bound2, norm2(tq, lo, hi) * norm2(tk, lo, hi))
        safe = bound2 * (1.1 * C * c_exp) ** 2 <= EXP_LIMIT ** 2
        flag_ref[0] = jnp.where(safe, 1, 0).astype(jnp.int32)
        os_ref[...] = jnp.ones(os_ref.shape, F32)
        qkv_ref[:, 4] = jnp.zeros((WS, WP, 128), U32)
        res_ref[...] = jnp.zeros(res_ref.shape, U32)
        if STATIC_PRO:
            for g in range(CW // 8):
                conv_group(g)
            for t in range(NTILE):
                xpose_tile(t, ln_tile(t))
        else:
            conv_only()
            ln_only()

    @pl.when((s > 0) & (s <= n_strips))
    def _():
        phase_b()
        safe = flag_ref[0] == 1

        @pl.when(safe)
        def _():
            attention_fast()

        @pl.when(jnp.logical_not(safe))
        def _():
            attention_exact()

    @pl.when(s == n_strips + 1)
    def _():
        out_only()


@jax.jit
def pallas_standalone__window_attn_davit__vision_kernel(
    x: jax.Array,
    dw_pe: jax.Array,
    w_qkv: jax.Array,
    w_o: jax.Array,
):
    B, H, W, Cc = x.shape
    assert B == 1 and Cc == C and dw_pe.shape == (3, 3, C)
    assert H % WS == 0 and W % WS == 0 and 384 < W <= 512
    n_strips = H // WS
    xt = jnp.transpose(x, (0, 1, 3, 2)).reshape(H, C, W)
    dw = dw_pe.reshape(9, C)

    strip = lambda a: jnp.minimum(a, n_strips - 1)
    full = lambda shape: pl.BlockSpec(shape, lambda a: (0,) * len(shape))
    out = pl.pallas_call(
        functools.partial(_kernel, n_strips=n_strips, width=W),
        grid=(n_strips + 2,),
        in_specs=[
            pl.BlockSpec((WS, C, 512), lambda a: (strip(a), 0, 0)),
            pl.BlockSpec((1, C, 512), lambda a: (jnp.maximum(strip(a) * WS - 1, 0), 0, 0)),
            pl.BlockSpec((1, C, 512), lambda a: (jnp.minimum(strip(a) * WS + WS, H - 1), 0, 0)),
            full((9, C)),
            full((C, 3 * C)),
            full((C, C)),
        ],
        out_specs=pl.BlockSpec((WS, C, 512), lambda a: (jnp.maximum(a - 2, 0), 0, 0)),
        out_shape=jax.ShapeDtypeStruct((H, C, W), x.dtype),
        scratch_shapes=[
            pltpu.VMEM((9, 2, CW, 128), F32),
            pltpu.VMEM((128, 640), U32),
            pltpu.VMEM((CW, 256), U32),
            pltpu.VMEM((WS, 2, CW, 512), F32),
            pltpu.VMEM((2, WS, CW, 512), U32),
            pltpu.VMEM((WS, 2, 256, 128), U32),
            pltpu.VMEM((WS, 6, 512, 128), U32),
            pltpu.VMEM((WS, 2, 512, 128), F32),
            pltpu.SMEM((1,), jnp.int32),
        ],
        compiler_params=pltpu.CompilerParams(
            dimension_semantics=("arbitrary",),
            vmem_limit_bytes=100 * 1024 * 1024,
            flags=FLAGS,
        ),
    )(xt, xt, xt, dw, w_qkv, w_o)
    return jnp.transpose(out.reshape(B, H, C, W), (0, 1, 3, 2))
```

```python
import functools

import jax
import jax.numpy as jnp
import jax.experimental.pallas as pl
import jax.experimental.pallas.tpu as pltpu
from jax import lax

WS = 7
NH = 4
C = 192
DH = C // NH
CW = C // 2
F32 = jnp.float32
BF16 = jnp.bfloat16
U32 = jnp.uint32
NT_DIMS = (((1,), (1,)), ((), ()))
NN_DIMS = (((1,), (0,)), ((), ()))
NEG = -1e30
LOG2E = 1.4426950408889634
EXP_LIMIT = 40.0
QORDER = (4, 0, 1, 2, 3)
SKEW = 2
FLAGS = {"XLA_TPU_EVENLY_DISTRIBUTE_CRITICAL_NODES": True}


def _dot(a, b, dims=NN_DIMS):
    return lax.dot_general(a, b, dims, preferred_element_type=F32)


def _iota(shape, dim):
    return lax.broadcasted_iota(jnp.int32, shape, dim)


def _f32(words):
    return pltpu.bitcast(words, F32)


def _lo(words):
    return _f32(words << 16)


def _hi(words):
    return _f32(words & U32(0xFFFF0000))


def _pack2(a, b):
    return pltpu.pack_elementwise([a, b], packed_dtype=BF16)


def _onehot(rows_map, cols_map):
    return jnp.where(rows_map == cols_map, 1.0, 0.0).astype(BF16)


def _prepare_weights(dw_ref, wqkv_ref, wo_ref, dwt_ref, wq_ref, wot_ref):
    r_i = _iota((CW, C), 0)
    c_i = _iota((CW, C), 1)
    for p in range(2):
        sel = _onehot(2 * r_i + p, c_i)
        for k in range(9):
            rep = jnp.broadcast_to(dw_ref[k:k + 1, :], (128, C))
            t = _dot(sel, rep, NT_DIMS)
            if k == 4:
                t = t + 1.0
            dwt_ref[k, p] = t
    rho = _iota((256, C), 0)
    rr = rho & 127
    chan = jnp.where(rr < CW, 2 * rr + (rho >> 7), -1)
    rsel = _onehot(chan, _iota((256, C), 1))
    w1 = _dot(rsel, wqkv_ref[...]).astype(BF16)
    n = _iota((3 * C, 640), 1)
    l = n & 127
    t = n >> 7
    col0 = jnp.where(l < 96, l, 384 + 64 + l - 96)
    col1 = jnp.where(l >= 32, 96 + l - 32, 384 + l)
    col2 = jnp.where(l < 96, 192 + l, -1)
    col3 = jnp.where(l >= 32, 288 + l - 32, -1)
    col4 = jnp.where(l < 32, 480 + l, jnp.where(l < 64, 384 + l, 448 + l))
    col = jnp.where(t == 0, col0, jnp.where(t == 1, col1, jnp.where(t == 2, col2,
                    jnp.where(t == 3, col3, col4))))
    csel = _onehot(_iota((3 * C, 640), 0), col)
    wq = _dot(w1, csel)
    wq_ref[...] = pltpu.bitcast(wq.astype(BF16), U32)
    lam = _iota((256, C), 0)
    ll = lam & 127
    fa = jnp.where(ll < 64, ll, jnp.where(ll < 96, -1, ll - 32))
    fb = jnp.where(ll < 32, 96 + ll, jnp.where(ll < 64, -1, 64 + ll))
    feat = jnp.where(lam < 128, fa, fb)
    fsel = _onehot(feat, _iota((256, C), 1))
    tmp = _dot(fsel, wo_ref[...]).astype(BF16)
    rp = _iota((C, C), 0)
    ochan = jnp.where(rp < CW, 2 * rp, 2 * (rp - CW) + 1)
    osel = _onehot(ochan, _iota((C, C), 1))
    wot_ref[...] = pltpu.bitcast(_dot(osel, tmp, NT_DIMS).astype(BF16), U32)


def _kernel(xm_ref, xt_ref, xb_ref, dw_ref, wqkv_ref, wo_ref, o_ref,
            dwt_ref, wq_ref, wot_ref, x0_ref, res_ref, hs_ref, qkv_ref, os_ref, flag_ref,
            *, n_strips, width):
    s = pl.program_id(0)
    WP = 512
    NTILE = WS * 4
    rslot = s & 1

    sub = _iota((8, 128), 0)
    lane = _iota((8, 128), 1)
    lo16, hi16 = U32(0x0000FFFF), U32(0xFFFF0000)
    zero = U32(0)

    def rows(m, n):
        return jnp.concatenate([m] * n, axis=0)

    def halves(hp0, hp1):
        return jnp.where(hp0, lo16, jnp.where(hp1, hi16, zero))

    key_ok = sub < WS
    kmask = [halves(lane < 48, (lane >= 48) & (lane < 96)),
             halves((lane >= 32) & (lane < 80), lane >= 80)]
    va1 = ((lane >= 48) & (lane < 64)) | (lane >= 96)
    vb1 = lane >= 80
    vmask = [halves(lane < 48, va1), halves((lane < 32) | ((lane >= 64) & (lane < 80)), vb1)]
    key_mask = jnp.where(key_ok, U32(0xFFFFFFFF), zero)
    one_lo, one_hi = U32(0x00003F80), U32(0x3F800000)

    def ones(d0):
        m = jnp.where((lane >= d0) & (lane < d0 + 16), one_lo,
                      jnp.where((lane >= d0 + 16) & (lane < d0 + 32), one_hi, zero))
        return m

    vones = [ones(64), ones(32)]
    den_idx = [jnp.where(va1, 80, 64), jnp.where(vb1, 48, 32)]
    even = (lane & 1) == 0
    s_valid = ((lane & 15) < 14) & (lane < 112)
    quarter = lane >> 5
    last_valid = lane < (width - 384)
    c_exp = (DH ** -0.5) * LOG2E

    def conv_steps(g):
        top_ok = s > 0
        bot_ok = s < n_strips - 1
        c0 = g * 16 if isinstance(g, int) else pl.multiple_of(g * 16, 16)
        r0 = g * 8 if isinstance(g, int) else pl.multiple_of(g * 8, 8)
        for p, unp in enumerate((_lo, _hi)):
            taps = [dwt_ref[k, p, pl.ds(r0, 8), :] for k in range(9)]
            xs = {}
            for r in range(-1, WS + 1):
                if r == -1:
                    raw = xt_ref[0, pl.ds(c0, 16), :]
                elif r == WS:
                    raw = xb_ref[0, pl.ds(c0, 16), :]
                else:
                    raw = xm_ref[r, pl.ds(c0, 16), :]
                w = pltpu.bitcast(raw, U32)
                w = jnp.concatenate([w[:, :384], jnp.where(last_valid, w[:, 384:], zero)], axis=1)
                if r == -1:
                    w = jnp.where(top_ok, w, zero)
                if r == WS:
                    w = jnp.where(bot_ok, w, zero)
                xs[r] = [unp(w[:, 128 * L:128 * L + 128]) for L in range(4)]
                if r >= 1:
                    i = r - 1
                    t = [jnp.concatenate(
                        [xs[i - 1][L] * taps[j] + xs[i][L] * taps[3 + j] + xs[i + 1][L] * taps[6 + j]
                         for L in range(4)], axis=1) for j in range(3)]
                    x0_ref[i, p, pl.ds(r0, 8), :] = (
                        pltpu.roll(t[0], 1, 1) + t[1] + pltpu.roll(t[2], WP - 1, 1))
                    del xs[i - 1]
                if p == 1:
                    yield

    def conv_group(g):
        for _ in conv_steps(g):
            pass

    def tile_pos(it):
        if isinstance(it, int):
            return it // 4, (it % 4) * 128
        return it >> 2, pl.multiple_of((it & 3) * 128, 128)

    def ln_tile(it):
        i, l0 = tile_pos(it)
        xe = x0_ref[i, 0, :, pl.ds(l0, 128)]
        xo = x0_ref[i, 1, :, pl.ds(l0, 128)]
        res_ref[rslot, i, :, pl.ds(l0, 128)] = _pack2(xe, xo)
        mean = jnp.sum(xe + xo, axis=0, keepdims=True) * (1.0 / C)
        de = xe - mean
        do = xo - mean
        var = jnp.sum(de * de + do * do, axis=0, keepdims=True) * (1.0 / C)
        rstd = lax.rsqrt(var + 1e-5)
        return _pack2(de * rstd, do * rstd)

    def xpose_tile(it, words):
        i, l0 = tile_pos(it)
        words = jnp.concatenate([words, jnp.zeros((128 - CW, 128), U32)], axis=0)
        words = words.T
        t0 = l0 // 2 if isinstance(l0, int) else pl.multiple_of(l0 >> 1, 64)
        for p, unp in enumerate((_lo, _hi)):
            hs_ref[i, p, pl.ds(t0, 64), :] = pltpu.bitcast(unp(words).astype(BF16), U32)

    def qkv_tile(it):
        i, l0 = tile_pos(it)
        t0 = l0 // 2 if isinstance(l0, int) else pl.multiple_of(l0 >> 1, 64)
        he = pltpu.bitcast(hs_ref[i, 0, pl.ds(t0, 64), :], BF16)
        ho = pltpu.bitcast(hs_ref[i, 1, pl.ds(t0, 64), :], BF16)
        q16 = rows(quarter, 16)
        dst = lambda j: qkv_ref.at[i, j, pl.ds(l0, 128), :]
        for j in QORDER:
            we = pltpu.bitcast(wq_ref[0:64, 128 * j:128 * (j + 1)], BF16)
            wo = pltpu.bitcast(wq_ref[64:128, 128 * j:128 * (j + 1)], BF16)
            t = _dot(he, we) + _dot(ho, wo)
            if j == 4:
                w = _pack2(t, t)
                dst(5)[...] = (w & rows(vmask[1], 16)) | rows(vones[1], 16)
                pltpu.store(dst(4), w & rows(vmask[0], 16), mask=q16 == 1)
                pltpu.store(dst(4), rows(vones[0], 16), mask=q16 == 2)
            elif j < 2:
                dst(j)[...] = pltpu.bitcast(t * c_exp, U32)
                pltpu.store(dst(4), _pack2(t, t) & rows(vmask[0], 16), mask=q16 == (3 if j == 0 else 0))
            else:
                dst(j)[...] = _pack2(t, t) & rows(kmask[j - 2], 16)

    zpad = jnp.zeros((16, 128), BF16)

    def gather(j, off):
        return jnp.concatenate([qkv_ref[i, j, pl.ds(off, 8), :] for i in range(WS)], axis=0)

    def scores(off, exact_max):
        ps = []
        for pr in range(2):
            q = _f32(gather(pr, off))
            kbd = jnp.concatenate([pltpu.bitcast(gather(2 + pr, off), BF16), zpad], axis=0)
            sc = _dot(q, kbd, NT_DIMS)
            if exact_max:
                sc = jnp.where(rows(s_valid, WS), sc, NEG)
                ev = rows(even, WS)
                m0 = jnp.max(jnp.where(ev, sc, NEG), axis=1, keepdims=True)
                m1 = jnp.max(jnp.where(ev, NEG, sc), axis=1, keepdims=True)
                sc = sc - jnp.where(ev, m0, m1)
            ps.append(jnp.exp2(sc))
        return ps

    def attend(off, ps):
        for pr in range(2):
            vw = gather(4 + pr, off) & rows(key_mask, WS)
            vbd = jnp.concatenate([pltpu.bitcast(vw, BF16), zpad], axis=0)
            o = _dot(ps[pr], vbd)
            for i in range(WS):
                os_ref[i, pr, pl.ds(off, 8), :] = o[8 * i:8 * i + 8, :]

    n_win = width // WS

    def attention(exact_max):
        steps = (xpose_tile(t, ln_tile(t)) for t in range(NTILE))
        n_steps = NTILE
        pend = [scores(WS * w, exact_max) for w in range(SKEW)]
        g = 0
        for w in range(n_win):
            if w + SKEW < n_win:
                pend.append(scores(WS * (w + SKEW), exact_max))
            attend(WS * w, pend.pop(0))
            while g * n_win < (w + 1) * n_steps:
                next(steps, None)
                g += 1
        for _ in steps:
            pass

    def out_load(it):
        i, l0 = tile_pos(it)
        ob = []
        for pr in range(2):
            o = os_ref[i, pr, pl.ds(l0, 128), :]
            den = jnp.take_along_axis(o, rows(den_idx[pr], 16), axis=1, mode="promise_in_bounds")
            ob.append((o * pltpu.reciprocal(den, approx=True, full_range=False)).astype(BF16))
        return ob, res_ref[rslot, i, :, pl.ds(l0, 128)]

    def out_tile(it, pre=None):
        i, l0 = tile_pos(it)
        (oa, ob), rw = out_load(it) if pre is None else pre
        wa = pltpu.bitcast(wot_ref[:, 0:128], BF16)
        wb = pltpu.bitcast(wot_ref[:, 128:256], BF16)
        y = _dot(wa, oa, NT_DIMS) + _dot(wb, ob, NT_DIMS)
        ye = y[0:CW] + _lo(rw)
        yo = y[CW:C] + _hi(rw)
        o_ref[i, :, pl.ds(l0, 128)] = pltpu.bitcast(_pack2(ye, yo), BF16)

    def out_only():
        for it in range(NTILE):
            out_tile(it)

    def phase_b():
        steps = (None for gg in range(CW // 8) for _ in conv_steps(gg))
        n_steps = (CW // 8) * (WS + 2)
        g = 0
        for it in range(NTILE):
            out_tile(it)
            qkv_tile(it)
            while g * NTILE < (it + 1) * n_steps:
                next(steps, None)
                g += 1
        for _ in steps:
            pass

    @pl.when(s == 0)
    def _():
        _prepare_weights(dw_ref, wqkv_ref, wo_ref, dwt_ref, wq_ref, wot_ref)
        wq = pltpu.bitcast(wq_ref[...], BF16).astype(F32)
        sq = jnp.sum(wq * wq, axis=0, keepdims=True)
        l640 = _iota((1, 640), 1)
        t640, l128 = l640 >> 7, l640 & 127

        def norm2(tile, lo, hi):
            return jnp.sum(jnp.where((t640 == tile) & (l128 >= lo) & (l128 < hi), sq, 0.0))
        heads = [(0, 2, 0, 48), (0, 2, 48, 96), (1, 3, 32, 80), (1, 3, 80, 128)]
        bound2 = 0.0
        for tq, tk, lo, hi in heads:
            bound2 = jnp.maximum(bound2, norm2(tq, lo, hi) * norm2(tk, lo, hi))
        safe = bound2 * (1.1 * C * c_exp) ** 2 <= EXP_LIMIT ** 2
        flag_ref[0] = jnp.where(safe, 1, 0).astype(jnp.int32)
        os_ref[...] = jnp.ones(os_ref.shape, F32)
        qkv_ref[:, 4] = jnp.zeros((WS, WP, 128), U32)
        res_ref[...] = jnp.zeros(res_ref.shape, U32)
        for g in range(CW // 8):
            conv_group(g)
        for t in range(NTILE):
            xpose_tile(t, ln_tile(t))

    @pl.when((s > 0) & (s <= n_strips))
    def _():
        phase_b()
        safe = flag_ref[0] == 1

        @pl.when(safe)
        def _():
            attention(False)

        @pl.when(jnp.logical_not(safe))
        def _():
            attention(True)

    @pl.when(s == n_strips + 1)
    def _():
        out_only()


@jax.jit
def pallas_standalone__window_attn_davit__vision_kernel(
    x: jax.Array,
    dw_pe: jax.Array,
    w_qkv: jax.Array,
    w_o: jax.Array,
):
    B, H, W, Cc = x.shape
    assert B == 1 and Cc == C and dw_pe.shape == (3, 3, C)
    assert H % WS == 0 and W % WS == 0 and 384 < W <= 512
    n_strips = H // WS
    xt = jnp.transpose(x, (0, 1, 3, 2)).reshape(H, C, W)
    dw = dw_pe.reshape(9, C)

    strip = lambda a: jnp.minimum(a, n_strips - 1)
    full = lambda shape: pl.BlockSpec(shape, lambda a: (0,) * len(shape))
    out = pl.pallas_call(
        functools.partial(_kernel, n_strips=n_strips, width=W),
        grid=(n_strips + 2,),
        in_specs=[
            pl.BlockSpec((WS, C, 512), lambda a: (strip(a), 0, 0)),
            pl.BlockSpec((1, C, 512), lambda a: (jnp.maximum(strip(a) * WS - 1, 0), 0, 0)),
            pl.BlockSpec((1, C, 512), lambda a: (jnp.minimum(strip(a) * WS + WS, H - 1), 0, 0)),
            full((9, C)),
            full((C, 3 * C)),
            full((C, C)),
        ],
        out_specs=pl.BlockSpec((WS, C, 512), lambda a: (jnp.maximum(a - 2, 0), 0, 0)),
        out_shape=jax.ShapeDtypeStruct((H, C, W), x.dtype),
        scratch_shapes=[
            pltpu.VMEM((9, 2, CW, 128), F32),
            pltpu.VMEM((128, 640), U32),
            pltpu.VMEM((CW, 256), U32),
            pltpu.VMEM((WS, 2, CW, 512), F32),
            pltpu.VMEM((2, WS, CW, 512), U32),
            pltpu.VMEM((WS, 2, 256, 128), U32),
            pltpu.VMEM((WS, 6, 512, 128), U32),
            pltpu.VMEM((WS, 2, 512, 128), F32),
            pltpu.SMEM((1,), jnp.int32),
        ],
        compiler_params=pltpu.CompilerParams(
            dimension_semantics=("arbitrary",),
            vmem_limit_bytes=100 * 1024 * 1024,
            flags=FLAGS,
        ),
    )(xt, xt, xt, dw, w_qkv, w_o)
    return jnp.transpose(out.reshape(B, H, C, W), (0, 1, 3, 2))
```
